```python
import jax
import jax.numpy as jnp

def _softmax(x, axis=-1):
    return jax.nn.softmax(x, axis=axis)

def _gelu(x):
    return jax.nn.gelu(x, approximate=True)

def _silu(x):
    return jax.nn.silu(x)

def _sigmoid(x):
    return jax.nn.sigmoid(x)

def _layernorm(x, axis=-1, eps=1e-05):
    m = jnp.mean(x, axis=axis, keepdims=True)
    v = jnp.var(x, axis=axis, keepdims=True)
    return (x - m) / jnp.sqrt(v + eps)

def _scatter_add(tgt, idx, src, axis=0):
    return tgt.at[idx].add(src)

def _segment_sum(src, seg, n):
    return jax.ops.segment_sum(src, seg, n)

class _Rng:

    def __init__(self, key):
        self._k = key

    def _next(self):
        self._k, sub = jax.random.split(self._k)
        return sub

    def normal(self, shape):
        return jax.random.normal(self._next(), shape, dtype=jnp.bfloat16)

    def randint(self, lo, hi, shape):
        return jax.random.randint(self._next(), shape, lo, hi, dtype=jnp.int32)

    def uniform(self, shape, lo=0.0, hi=1.0):
        return jax.random.uniform(self._next(), shape, jnp.bfloat16, lo, hi)

    def permutation(self, n):
        return jax.random.permutation(self._next(), n)
kernel_name = 'adaLN_cond__memory_aug_recurrent_mem_tr__mixer_s_mlp__prompt'

def setup_inputs():
    _rng = _Rng(jax.random.key(int.from_bytes(__import__("os").urandom(4), "little")))
    _w = lambda a: (lambda t: t.astype(jnp.bfloat16) if jnp.issubdtype(t.dtype, jnp.floating) else t)(jnp.asarray(a))

    def _A_setup():
        B, S, Dm = (1, 2048, 1024)
        H, Dh = (32, 128)
        M, seg = (8, 32)
        seg = min(seg, S)
        S = S // seg * seg
        return {'x': _w((lambda *s: _rng.normal(s) * 0.05)(B, S, Dm)), 'mem0': _w((lambda *s: _rng.normal(s) * 0.05)(B, M, Dm)), 'Wq': _w((lambda *s: _rng.normal(s) * 0.05)(Dm, H, Dh) * Dm ** (-0.5)), 'Wk': _w((lambda *s: _rng.normal(s) * 0.05)(Dm, H, Dh) * Dm ** (-0.5)), 'Wv': _w((lambda *s: _rng.normal(s) * 0.05)(Dm, H, Dh) * Dm ** (-0.5)), 'Wo': _w((lambda *s: _rng.normal(s) * 0.05)(H, Dh, Dm) * (H * Dh) ** (-0.5)), 'seg_len': seg}
    _A_in = _A_setup()

    def _B_setup():
        B, S, D, F = (1, 2048, 1024, 3584)
        return {'x': _w((lambda *s: _rng.normal(s) * 0.05)(B, S, D)), 'w1': _w((lambda *s: _rng.normal(s) * 0.05)(D, D) * D ** (-0.5)), 'w2': _w((lambda *s: _rng.normal(s) * 0.05)(D, D) * D ** (-0.5)), 'w3': _w((lambda *s: _rng.normal(s) * 0.05)(D, F) * D ** (-0.5)), 'w4': _w((lambda *s: _rng.normal(s) * 0.05)(F, D) * F ** (-0.5))}
    _B_in = _B_setup()
    return {'A_x': _A_in['x'], 'A_mem0': _A_in['mem0'], 'A_Wq': _A_in['Wq'], 'A_Wk': _A_in['Wk'], 'A_Wv': _A_in['Wv'], 'A_Wo': _A_in['Wo'], 'A_seg_len': _A_in['seg_len'], 'B_x': _B_in['x'], 'B_w1': _B_in['w1'], 'B_w2': _B_in['w2'], 'B_w3': _B_in['w3'], 'B_w4': _B_in['w4'], 'c': _w((lambda *s: _rng.normal(s) * 0.05)(1, 1024)), 'w_mod': _w((lambda *s: _rng.normal(s) * 0.05)(1024, 6 * 1024) * 1024 ** (-0.5))}

def reference(A_x, A_mem0, A_Wq, A_Wk, A_Wv, A_Wo, A_seg_len, B_x, B_w1, B_w2, B_w3, B_w4, c, w_mod):

    def _A_ref(x, mem0, Wq, Wk, Wv, Wo, seg_len):
        B, S, Dm = x.shape
        H, Dh = (Wq.shape[1], Wq.shape[2])
        M = mem0.shape[1]
        scale = Dh ** (-0.5)
        n_seg = S // seg_len
        L = M + seg_len
        idx = jnp.arange(L)
        mask = (idx[:, None] < M) | (idx[:, None] >= idx[None, :])
        mem = mem0
        outs = []
        for s in range(n_seg):
            xs = x[:, s * seg_len:(s + 1) * seg_len, :].copy()
            h = jnp.concatenate([mem, xs], axis=1)
            q = jnp.einsum('btd,dhe->bhte', h, Wq)
            k = jnp.einsum('btd,dhe->bhte', h, Wk)
            v = jnp.einsum('btd,dhe->bhte', h, Wv)
            scores = jnp.einsum('bhqe,bhke->bhqk', q, k) * scale
            scores = jnp.where(mask[None, None], scores, -1000000000.0)
            p = _softmax(scores, axis=-1)
            o = jnp.einsum('bhqk,bhke->bhqe', p, v)
            o = jnp.einsum('bhte,hed->btd', o, Wo)
            mem = o[:, :M, :].copy()
            outs.append(o[:, M:, :])
        return jnp.concatenate(outs, axis=1)

    def _B_ref(x, w1, w2, w3, w4):
        B, S, D = x.shape
        h = _gelu(_layernorm(x, axis=-1) @ w1)
        c = D // 4
        g0 = jnp.pad(h[:, :, 0 * c:1 * c], ((0, 0), (1, 0), (0, 0)))[:, :S, :]
        g1 = jnp.pad(h[:, :, 1 * c:2 * c], ((0, 0), (0, 1), (0, 0)))[:, 1:, :]
        g2 = jnp.pad(h[:, :, 2 * c:3 * c], ((0, 0), (2, 0), (0, 0)))[:, :S, :]
        g3 = jnp.pad(h[:, :, 3 * c:], ((0, 0), (0, 2), (0, 0)))[:, 2:, :]
        hs = jnp.concatenate([g0, g1, g2, g3], axis=-1) @ w2
        x1 = x + hs
        h2 = _gelu(_layernorm(x1, axis=-1) @ w3) @ w4
        return x1 + h2
    x = A_x
    mod = (_silu(c) @ w_mod).reshape(c.shape[0], 6, 1, -1)
    sa, ca, ga, sb, cb, gb = (mod[:, 0].copy(), mod[:, 1].copy(), mod[:, 2].copy(), mod[:, 3].copy(), mod[:, 4].copy(), mod[:, 5].copy())
    h = _layernorm(x, axis=-1) * (1 + ca) + sa
    x = x + ga * _A_ref(h, A_mem0, A_Wq, A_Wk, A_Wv, A_Wo, A_seg_len)
    h = _layernorm(x, axis=-1) * (1 + cb) + sb
    x = x + gb * _B_ref(h, B_w1, B_w2, B_w3, B_w4)
    return x
```

```python
import functools

import jax
import jax.numpy as jnp
import jax.experimental.pallas as pl
import jax.experimental.pallas.tpu as pltpu

F32 = jnp.float32
BF16 = jnp.bfloat16
U32 = jnp.uint32
LANE = 128


def _dot(a, b):
    return jax.lax.dot_general(a, b, (((1,), (0,)), ((), ())), preferred_element_type=F32)


def _dot_nt(a, b):
    return jax.lax.dot_general(a, b, (((1,), (1,)), ((), ())), preferred_element_type=F32)


def _ln(x):
    m = jnp.mean(x, axis=-1, keepdims=True)
    xc = x - m
    v = jnp.mean(xc * xc, axis=-1, keepdims=True)
    return xc * jax.lax.rsqrt(v + 1e-5)


def _gelu(x):
    return jax.nn.gelu(x, approximate=True)


def _make_kernel(S, D, H, M, SEG, F):
    NSEG = S // SEG
    R = SEG - M
    P = S - R * NSEG
    RING = 576
    OFF = RING - P
    L = SEG + M
    HC = 16
    NCD = D // LANE
    BM = 512
    FC = 512
    PAD = 32
    scale = float(LANE) ** -0.5

    def kernel(x_hbm, mem0_ref, wq_hbm, wk_hbm, wv_hbm, wo_hbm, w1_hbm, w2_hbm, w3_hbm, w4_hbm, c_ref, wmod_hbm,
               out_hbm,
               x_s, h_s, wqkv_s, wo_s, w1_s, w2_s, w3_s, w4_s, wmod_s, stage_s, ring_s, mod_s, lhs_s, o_s, a_s,
               g_s, acc_s, ln_s, y_s, ob_s, sems):
        sem_i = iter(range(64))

        def copy(src, dst):
            return pltpu.make_async_copy(src, dst, sems.at[next(sem_i)])

        def wmod_copy(j, slot):
            return copy(wmod_hbm.at[:, pl.ds(2 * D * j, 2 * D)], wmod_s.at[slot])

        cp_mod = [wmod_copy(0, 0), wmod_copy(1, 1), wmod_copy(2, 0)]
        cp_x0 = copy(x_hbm.at[pl.ds(0, P)], x_s.at[pl.ds(PAD, P)])
        cp_x1 = copy(x_hbm.at[pl.ds(P, S - P)], x_s.at[pl.ds(PAD + P, S - P)])
        chunks = [(w, t, hc) for t, w in enumerate((wq_hbm, wk_hbm, wv_hbm)) for hc in range(H // HC)]
        NST = stage_s.shape[0]
        cp_w = [copy(w.at[:, pl.ds(hc * HC, HC), :], stage_s.at[i % NST]) for i, (w, t, hc) in enumerate(chunks)]
        cp_wo = [copy(wo_hbm.at[:, pl.ds(j * LANE, LANE)], wo_s.at[j]) for j in range(NCD)]
        cp_w1 = [copy(w1_hbm.at[:, pl.ds(j * LANE, LANE)], w1_s.at[j]) for j in range(NCD)]
        cp_w2 = copy(w2_hbm, w2_s)
        cp_w3 = [copy(w3_hbm.at[:, pl.ds(j * FC, FC)], w3_s.at[j]) for j in range(F // FC)]
        cp_w4 = copy(w4_hbm, w4_s)

        cp_mod[0].start()
        cp_x0.start()
        for i in range(NST):
            cp_w[i].start()

        cv = jnp.broadcast_to(c_ref[...].astype(F32), (8, D))
        sc = cv * jax.nn.sigmoid(cv)

        def do_mod(j, slot):
            cp_mod[j].wait()
            mod_s[:, pl.ds(2 * D * j, 2 * D)] = _dot(sc, wmod_s[slot])

        def mod(i):
            return mod_s[pl.ds(0, 1), pl.ds(i * D, D)]

        x_s[pl.ds(0, PAD), :] = jnp.zeros((PAD, D), BF16)
        a_s[...] = jnp.zeros(a_s.shape, F32)
        g_s[pl.ds(PAD + S, 8), :] = jnp.zeros((8, D), F32)

        do_mod(0, 0)
        cp_x0.wait()

        def adaln_rows(r0, n, rows):
            def body(i, carry):
                r = pl.multiple_of(PAD + r0 + i * rows, 32)
                xv = x_s[pl.ds(r, rows), :].astype(F32)
                h_s[pl.ds(r, rows), :] = (_ln(xv) * (1.0 + mod(1)) + mod(0)).astype(BF16)
                return carry
            jax.lax.fori_loop(0, n // rows, body, 0)

        adaln_rows(0, P, 64)

        for i, (w, t, hc) in enumerate(chunks):
            cp_w[i].wait()
            base = t * H + hc * HC

            def relayout(k, carry, i=i, base=base):
                v = stage_s[i % NST, pl.ds(pl.multiple_of(k * 32, 32), 32), :, :]
                v = pltpu.bitcast(v, U32).reshape(16, 2, HC // 2, LANE)
                a = jnp.swapaxes(v[:, 0], 0, 1)
                b = jnp.swapaxes(v[:, 1], 0, 1)
                lo = (a & 0xFFFF) | (b << 16)
                hi = (a >> 16) | ((b >> 16) << 16)
                rows = pl.ds(pl.multiple_of(k * 32, 32), 32)
                for j in range(HC // 2):
                    wqkv_s[base + 2 * j, rows, :] = pltpu.bitcast(lo[j], BF16)
                    wqkv_s[base + 2 * j + 1, rows, :] = pltpu.bitcast(hi[j], BF16)
                return carry
            jax.lax.fori_loop(0, D // 32, relayout, 0)
            if i + NST < len(chunks):
                cp_w[i + NST].start()
            if i + NST == len(chunks) - 1:
                cp_x1.start()
                cp_mod[1].start()
                cp_mod[2].start()
                for cp in cp_wo + cp_w1 + [cp_w2] + cp_w3 + [cp_w4]:
                    cp.start()

            def bulk(k, carry, base=base):
                lhs = h_s[pl.ds(PAD, P), :]
                for u in range(4):
                    j = base + k * 4 + u
                    ring_s[j, pl.ds(OFF, P), :] = _dot(lhs, wqkv_s[j]).astype(BF16)
                return carry
            jax.lax.fori_loop(0, HC // 4, bulk, 0)

        cp_x1.wait()
        adaln_rows(P, S - P, 64)
        do_mod(1, 1)
        do_mod(2, 0)
        for cp in cp_wo + cp_w1:
            cp.wait()

        lhs_s[...] = mem0_ref[...].astype(F32)

        row = jax.lax.broadcasted_iota(jnp.int32, (L, L), 0)
        col = jax.lax.broadcasted_iota(jnp.int32, (L, L), 1)

        def post_attention(r):
            x1 = (x_s[pl.ds(r, SEG), :].astype(F32) + mod(2) * a_s[...]).astype(BF16)
            x_s[pl.ds(r, SEG), :] = x1
            h2 = (_ln(x1.astype(F32)) * (1.0 + mod(4)) + mod(3)).astype(BF16)
            h_s[pl.ds(r, SEG), :] = h2
            n2 = _ln(h2.astype(F32)).astype(BF16)
            return n2

        def w1_stage(n2, r):
            for j in range(NCD):
                g_s[pl.ds(r, SEG), pl.ds(j * LANE, LANE)] = _gelu(_dot(n2, w1_s[j]))

        def step(s, carry):
            mask = (row >= SEG) | (col >= SEG) | (row >= col)
            wpos = pl.multiple_of(jax.lax.rem(s * R, RING), 8)
            rpos = pl.multiple_of(jax.lax.rem(s * SEG + OFF, RING), SEG)
            tok = h_s[pl.ds(pl.multiple_of(PAD + P + s * R, 8), R), :].astype(F32)
            lhs = jnp.concatenate([tok, lhs_s[...]], axis=0).astype(BF16)
            prev = pl.multiple_of(PAD + (s - 1) * SEG, SEG)
            n2 = post_attention(prev)

            def proj(j):
                y = _dot(lhs, wqkv_s[j])
                ring_s[j, pl.ds(wpos, R), :] = y[:R].astype(BF16)
                return y[R:]

            def full(j, m):
                return jnp.concatenate([ring_s[j, pl.ds(rpos, SEG), :].astype(F32), m], axis=0)

            qm, km, vm, pr = {}, {}, {}, {}
            for i in range(H + 2):
                if 0 <= i - 1 < H:
                    q = full(i - 1, qm.pop(i - 1))
                    k = full(H + i - 1, km.pop(i - 1))
                if 0 <= i - 2 < H:
                    v = full(2 * H + i - 2, vm.pop(i - 2))
                if i < H:
                    qm[i] = proj(i)
                if 0 <= i - 1 < H:
                    sco = jnp.where(mask, _dot_nt(q, k) * scale, -1e9)
                    e = jnp.exp(sco - jnp.max(sco, axis=-1, keepdims=True))
                    pr[i - 1] = e / jnp.sum(e, axis=-1, keepdims=True)
                if i < H:
                    km[i] = proj(H + i)
                    vm[i] = proj(2 * H + i)
                if i == H:
                    w1_stage(n2, prev)
                if 0 <= i - 2 < H:
                    o_s[:, pl.ds((i - 2) * LANE, LANE)] = _dot(pr.pop(i - 2), v)
            for j in range(NCD):
                y = _dot(o_s[...], wo_s[j])
                a_s[:, pl.ds(j * LANE, LANE)] = y[:SEG]
                lhs_s[:, pl.ds(j * LANE, LANE)] = y[SEG:]
            return carry

        jax.lax.fori_loop(0, NSEG, step, 0)
        last = PAD + S - SEG
        w1_stage(post_attention(last), last)
        g_s[pl.ds(PAD - 8, 8), :] = jnp.zeros((8, D), F32)

        for cp in [cp_w2] + cp_w3 + [cp_w4]:
            cp.wait()

        osem = next(sem_i)

        def out_copy(b):
            return pltpu.make_async_copy(ob_s, out_hbm.at[pl.ds(pl.multiple_of(b * BM, BM), BM)], sems.at[osem])

        Q = D // 4

        def block(b, carry):
            r = pl.multiple_of(PAD + b * BM, 32)
            parts = []
            for gi, sh in enumerate((-1, 1, -2, 2)):
                gv = g_s[pl.ds(pl.multiple_of(r - 8, 8), BM + 16), pl.ds(gi * Q, Q)]
                parts.append(gv[8 + sh:8 + sh + BM].astype(BF16))
            y1 = h_s[pl.ds(r, BM), :].astype(F32) + _dot(jnp.concatenate(parts, axis=1), w2_s[...])
            acc_s[...] = y1
            ln_s[...] = _ln(y1).astype(BF16)

            def mlp(f, carry):
                u = _gelu(_dot(ln_s[...], w3_s[f])).astype(BF16)
                acc_s[...] += _dot(u, w4_s[pl.ds(pl.multiple_of(f * FC, FC), FC), :])
                return carry
            jax.lax.fori_loop(0, F // FC, mlp, 0)

            @pl.when(b > 0)
            def _():
                out_copy(b - 1).wait()
            ob_s[...] = (x_s[pl.ds(r, BM), :].astype(F32) + mod(5) * acc_s[...]).astype(BF16)
            out_copy(b).start()
            return carry

        jax.lax.fori_loop(0, S // BM, block, 0)
        out_copy(S // BM - 1).wait()

    scratch = [
        pltpu.VMEM((PAD + S, D), BF16),
        pltpu.VMEM((PAD + S, D), BF16),
        pltpu.VMEM((3 * H, D, LANE), BF16),
        pltpu.VMEM((NCD, H * LANE, LANE), BF16),
        pltpu.VMEM((NCD, D, LANE), BF16),
        pltpu.VMEM((D, D), BF16),
        pltpu.VMEM((F // FC, D, FC), BF16),
        pltpu.VMEM((F, D), BF16),
        pltpu.VMEM((2, D, 2 * D), BF16),
        pltpu.VMEM((3, D, HC, LANE), BF16),
        pltpu.VMEM((3 * H, RING, LANE), BF16),
        pltpu.VMEM((8, 6 * D), F32),
        pltpu.VMEM((M, D), F32),
        pltpu.VMEM((L, H * LANE), F32),
        pltpu.VMEM((SEG, D), F32),
        pltpu.VMEM((PAD + S + 8, D), F32),
        pltpu.VMEM((BM, D), F32),
        pltpu.VMEM((BM, D), BF16),
        pltpu.VMEM((8, LANE), F32),
        pltpu.VMEM((BM, D), BF16),
        pltpu.SemaphoreType.DMA((64,)),
    ]
    return kernel, scratch


@functools.partial(jax.jit, static_argnames=("A_seg_len",))
def pallas_adaLN_cond__memory_aug_recurrent_mem_tr__mixer_s_mlp__prompt_kernel(
    A_x: jax.Array,
    A_mem0: jax.Array,
    A_Wq: jax.Array,
    A_Wk: jax.Array,
    A_Wv: jax.Array,
    A_Wo: jax.Array,
    A_seg_len: int,
    B_x: jax.Array,
    B_w1: jax.Array,
    B_w2: jax.Array,
    B_w3: jax.Array,
    B_w4: jax.Array,
    c: jax.Array,
    w_mod: jax.Array,
):
    del B_x
    B, S, D = A_x.shape
    _, H, Dh = A_Wq.shape
    M = A_mem0.shape[1]
    F = B_w3.shape[1]
    assert B == 1 and Dh == LANE
    kernel, scratch = _make_kernel(S, D, H, M, int(A_seg_len), F)
    hbm = pl.BlockSpec(memory_space=pl.ANY)
    vmem = pl.BlockSpec(memory_space=pltpu.VMEM)
    out = pl.pallas_call(
        kernel,
        in_specs=[hbm, vmem, hbm, hbm, hbm, hbm, hbm, hbm, hbm, hbm, vmem, hbm],
        out_specs=hbm,
        out_shape=jax.ShapeDtypeStruct((S, D), A_x.dtype),
        scratch_shapes=scratch,
        compiler_params=pltpu.CompilerParams(vmem_limit_bytes=127 * 1024 * 1024),
    )(A_x.reshape(S, D), A_mem0.reshape(M, D), A_Wq, A_Wk, A_Wv, A_Wo.reshape(H * Dh, D),
      B_w1, B_w2, B_w3, B_w4, c, w_mod)
    return out.reshape(B, S, D)
```

```python
import functools

import jax
import jax.numpy as jnp
import jax.experimental.pallas as pl
import jax.experimental.pallas.tpu as pltpu

F32 = jnp.float32
BF16 = jnp.bfloat16
U32 = jnp.uint32
LANE = 128
CFG = dict(qk=2, v=3, pv=5, post=0)


def _dot(a, b):
    return jax.lax.dot_general(a, b, (((1,), (0,)), ((), ())), preferred_element_type=F32)


def _dot_nt(a, b):
    return jax.lax.dot_general(a, b, (((1,), (1,)), ((), ())), preferred_element_type=F32)


def _bf(w):
    return pltpu.bitcast(w, BF16)


def _ln(x):
    m = jnp.mean(x, axis=-1, keepdims=True)
    xc = x - m
    v = jnp.mean(xc * xc, axis=-1, keepdims=True)
    return xc * jax.lax.rsqrt(v + 1e-5)


def _gelu(x):
    return jax.nn.gelu(x, approximate=True)


def _make_kernel(S, D, H, M, SEG, F):
    NSEG = S // SEG
    R = SEG - M
    P = S - R * NSEG
    RING = 576
    OFF = RING - P
    L = SEG + M
    HC = 16
    NCD = D // LANE
    BM = 512
    FC = 512
    PAD = 32
    LAG_QK, LAG_V, LAG_PV = CFG['qk'], CFG['v'], CFG['pv']
    scale = float(LANE) ** -0.5

    def kernel(x_hbm, mem0_ref, wq_hbm, wk_hbm, wv_hbm, wo_hbm, w1_hbm, w2_hbm, w3_hbm, w4_hbm, c_ref, wmod_hbm,
               out_hbm,
               x_s, h_s, wqkv_s, wo_s, w1_s, w2_s, w3_s, w4_s, wmod_s, stage_s, ring_s, mod_s, lhs_s, o_s, a_s,
               g_s, acc_s, ln_s, y_s, ob_s, sems):
        sem_i = iter(range(64))

        def copy(src, dst):
            return pltpu.make_async_copy(src, dst, sems.at[next(sem_i)])

        def wmod_copy(j, slot):
            return copy(wmod_hbm.at[:, pl.ds(2 * D * j, 2 * D)], wmod_s.at[slot].bitcast(BF16))

        cp_mod = [wmod_copy(0, 0), wmod_copy(1, 1), wmod_copy(2, 0)]
        cp_x0 = copy(x_hbm.at[pl.ds(0, P)], x_s.at[pl.ds(PAD, P)])
        cp_x1 = copy(x_hbm.at[pl.ds(P, S - P)], x_s.at[pl.ds(PAD + P, S - P)])
        chunks = [(w, t, hc) for t, w in enumerate((wq_hbm, wk_hbm, wv_hbm)) for hc in range(H // HC)]
        NST = stage_s.shape[0]
        cp_w = [copy(w.at[:, pl.ds(hc * HC, HC), :], stage_s.at[i % NST]) for i, (w, t, hc) in enumerate(chunks)]
        cp_wo = [copy(wo_hbm, wo_s.bitcast(BF16))]
        cp_w1 = [copy(w1_hbm, w1_s.bitcast(BF16))]
        cp_w2 = copy(w2_hbm, w2_s.bitcast(BF16))
        cp_w3 = [copy(w3_hbm.at[:, pl.ds(j * FC, FC)], w3_s.at[j].bitcast(BF16)) for j in range(F // FC)]
        cp_w4 = copy(w4_hbm, w4_s.bitcast(BF16))

        cp_mod[0].start()
        cp_x0.start()
        for i in range(NST):
            cp_w[i].start()

        cv = jnp.broadcast_to(c_ref[...].astype(F32), (8, D))
        sc = cv * jax.nn.sigmoid(cv)

        def do_mod(j, slot):
            cp_mod[j].wait()
            mod_s[:, pl.ds(2 * D * j, 2 * D)] = _dot(sc, _bf(wmod_s[slot]))

        def mod(i):
            return mod_s[pl.ds(0, 1), pl.ds(i * D, D)]

        x_s[pl.ds(0, PAD), :] = jnp.zeros((PAD, D), BF16)
        a_s[...] = jnp.zeros(a_s.shape, F32)
        y_s[...] = jnp.zeros(y_s.shape, U32)
        g_s[pl.ds(PAD + S, 8), :] = jnp.zeros((8, D), F32)

        do_mod(0, 0)
        cp_x0.wait()

        def adaln_rows(r0, n, rows):
            def body(i, carry):
                r = pl.multiple_of(PAD + r0 + i * rows, 32)
                xv = x_s[pl.ds(r, rows), :].astype(F32)
                h_s[pl.ds(r, rows), :] = (_ln(xv) * (1.0 + mod(1)) + mod(0)).astype(BF16)
                return carry
            jax.lax.fori_loop(0, n // rows, body, 0)

        adaln_rows(0, P, 64)

        for i, (w, t, hc) in enumerate(chunks):
            cp_w[i].wait()
            base = t * H + hc * HC

            def relayout(k, carry, i=i, base=base):
                v = stage_s[i % NST, pl.ds(pl.multiple_of(k * 32, 32), 32), :, :]
                v = pltpu.bitcast(v, U32).reshape(16, 2, HC // 2, LANE)
                a = jnp.swapaxes(v[:, 0], 0, 1)
                b = jnp.swapaxes(v[:, 1], 0, 1)
                lo = (a & 0xFFFF) | (b << 16)
                hi = (a >> 16) | ((b >> 16) << 16)
                rows = pl.ds(pl.multiple_of(k * 16, 16), 16)
                for j in range(HC // 2):
                    wqkv_s[base + 2 * j, rows, :] = lo[j]
                    wqkv_s[base + 2 * j + 1, rows, :] = hi[j]
                return carry
            jax.lax.fori_loop(0, D // 32, relayout, 0)
            if i + NST < len(chunks):
                cp_w[i + NST].start()
            if i + NST == len(chunks) - 1:
                cp_x1.start()
                cp_mod[1].start()
                cp_mod[2].start()
                for cp in cp_wo + cp_w1 + [cp_w2] + cp_w3 + [cp_w4]:
                    cp.start()

            def bulk(k, carry, base=base):
                lhs = h_s[pl.ds(PAD, P), :]
                for u in range(4):
                    j = base + k * 4 + u
                    ring_s[j, pl.ds(OFF, P), :] = _dot(lhs, _bf(wqkv_s[j])).astype(BF16)
                return carry
            jax.lax.fori_loop(0, HC // 4, bulk, 0)

        cp_x1.wait()
        adaln_rows(P, S - P, 64)
        do_mod(1, 1)
        do_mod(2, 0)
        for cp in cp_wo + cp_w1:
            cp.wait()

        lhs_s[...] = mem0_ref[...].astype(F32)

        row = jax.lax.broadcasted_iota(jnp.int32, (L, L), 0)
        col = jax.lax.broadcasted_iota(jnp.int32, (L, L), 1)

        def post_attention(r):
            x1 = (x_s[pl.ds(r, SEG), :].astype(F32) + mod(2) * a_s[...]).astype(BF16)
            x_s[pl.ds(r, SEG), :] = x1
            h2 = (_ln(x1.astype(F32)) * (1.0 + mod(4)) + mod(3)).astype(BF16)
            h_s[pl.ds(r, SEG), :] = h2
            n2 = _ln(h2.astype(F32)).astype(BF16)
            return n2

        def w1_stage(n2, r):
            for j in range(NCD):
                g_s[pl.ds(r, SEG), pl.ds(j * LANE, LANE)] = _gelu(_dot(n2, _bf(w1_s[:, pl.ds(j * LANE, LANE)])))

        def step(s, carry):
            mask = (row >= SEG) | (col >= SEG) | (row >= col)
            wpos = pl.multiple_of(jax.lax.rem(s * R, RING), 8)
            rpos = pl.multiple_of(jax.lax.rem(s * SEG + OFF, RING), SEG)
            tok = h_s[pl.ds(pl.multiple_of(PAD + P + s * R, 8), R), :].astype(F32)
            lhs = jnp.concatenate([tok, lhs_s[...]], axis=0).astype(BF16)
            prev = pl.multiple_of(PAD + (s - 1) * SEG, SEG)
            n2 = post_attention(prev)

            def proj(j):
                y = _dot(lhs, _bf(wqkv_s[j]))
                ring_s[j, pl.ds(wpos, R), :] = y[:R].astype(BF16)
                return y[R:]

            def full(j, m):
                return jnp.concatenate([ring_s[j, pl.ds(rpos, SEG), :].astype(F32), m], axis=0)

            qs, ks, vs, pr = {}, {}, {}, {}
            for i in range(H + LAG_PV):
                if i < H:
                    qm = proj(i)
                if 0 <= i - LAG_QK < H:
                    hq = i - LAG_QK
                    sco = jnp.where(mask, _dot_nt(qs.pop(hq), ks.pop(hq)) * scale, -1e9)
                    e = jnp.exp(sco - jnp.max(sco, axis=-1, keepdims=True))
                    pr[hq] = e if CFG['post'] else e / jnp.sum(e, axis=-1, keepdims=True)
                if i < H:
                    km = proj(H + i)
                    qs[i] = full(i, qm)
                    ks[i] = full(H + i, km)
                if 0 <= i - LAG_V < H:
                    hv = i - LAG_V
                    vs[hv] = full(2 * H + hv, proj(2 * H + hv))
                if i == H + LAG_V:
                    w1_stage(n2, prev)
                if 0 <= i - LAG_PV < H:
                    hp = i - LAG_PV
                    e = pr.pop(hp)
                    o = _dot(e, vs.pop(hp))
                    if CFG['post']:
                        o = o * (1.0 / jnp.sum(e, axis=-1, keepdims=True))
                    o_s[:, pl.ds(hp * LANE, LANE)] = o
            for j in range(NCD):
                y = _dot(o_s[...], _bf(wo_s[:, pl.ds(j * LANE, LANE)]))
                a_s[:, pl.ds(j * LANE, LANE)] = y[:SEG]
                lhs_s[:, pl.ds(j * LANE, LANE)] = y[SEG:]
            return carry

        jax.lax.fori_loop(0, NSEG, step, 0)
        last = PAD + S - SEG
        w1_stage(post_attention(last), last)
        g_s[pl.ds(PAD - 8, 8), :] = jnp.zeros((8, D), F32)

        for cp in [cp_w2] + cp_w3 + [cp_w4]:
            cp.wait()

        osem = next(sem_i)

        def out_copy(b):
            return pltpu.make_async_copy(ob_s, out_hbm.at[pl.ds(pl.multiple_of(b * BM, BM), BM)], sems.at[osem])

        Q = D // 4

        def block(b, carry):
            r = pl.multiple_of(PAD + b * BM, 32)
            parts = []
            for gi, sh in enumerate((-1, 1, -2, 2)):
                gv = g_s[pl.ds(pl.multiple_of(r - 8, 8), BM + 16), pl.ds(gi * Q, Q)]
                parts.append(gv[8 + sh:8 + sh + BM].astype(BF16))
            y1 = h_s[pl.ds(r, BM), :].astype(F32) + _dot(jnp.concatenate(parts, axis=1), _bf(w2_s[...]))
            acc_s[...] = y1
            ln_s[...] = _ln(y1).astype(BF16)

            def mlp(f, carry):
                u = _gelu(_dot(ln_s[...], _bf(w3_s[f]))).astype(BF16)
                acc_s[...] += _dot(u, _bf(w4_s[pl.ds(pl.multiple_of(f * (FC // 2), FC // 2), FC // 2), :]))
                return carry
            jax.lax.fori_loop(0, F // FC, mlp, 0)

            @pl.when(b > 0)
            def _():
                out_copy(b - 1).wait()
            ob_s[...] = (x_s[pl.ds(r, BM), :].astype(F32) + mod(5) * acc_s[...]).astype(BF16)
            out_copy(b).start()
            return carry

        jax.lax.fori_loop(0, S // BM, block, 0)
        out_copy(S // BM - 1).wait()

    scratch = [
        pltpu.VMEM((PAD + S, D), BF16),
        pltpu.VMEM((PAD + S, D), BF16),
        pltpu.VMEM((3 * H, D // 2, LANE), U32),
        pltpu.VMEM((H * LANE // 2, D), U32),
        pltpu.VMEM((D // 2, D), U32),
        pltpu.VMEM((D // 2, D), U32),
        pltpu.VMEM((F // FC, D // 2, FC), U32),
        pltpu.VMEM((F // 2, D), U32),
        pltpu.VMEM((2, D // 2, 2 * D), U32),
        pltpu.VMEM((3, D, HC, LANE), BF16),
        pltpu.VMEM((3 * H, RING, LANE), BF16),
        pltpu.VMEM((8, 6 * D), F32),
        pltpu.VMEM((M, D), F32),
        pltpu.VMEM((L, H * LANE), F32),
        pltpu.VMEM((SEG, D), F32),
        pltpu.VMEM((PAD + S + 8, D), F32),
        pltpu.VMEM((BM, D), F32),
        pltpu.VMEM((BM, D), BF16),
        pltpu.VMEM((8, LANE), U32),
        pltpu.VMEM((BM, D), BF16),
        pltpu.SemaphoreType.DMA((64,)),
    ]
    return kernel, scratch


@functools.partial(jax.jit, static_argnames=("A_seg_len",))
def pallas_adaLN_cond__memory_aug_recurrent_mem_tr__mixer_s_mlp__prompt_kernel(
    A_x: jax.Array,
    A_mem0: jax.Array,
    A_Wq: jax.Array,
    A_Wk: jax.Array,
    A_Wv: jax.Array,
    A_Wo: jax.Array,
    A_seg_len: int,
    B_x: jax.Array,
    B_w1: jax.Array,
    B_w2: jax.Array,
    B_w3: jax.Array,
    B_w4: jax.Array,
    c: jax.Array,
    w_mod: jax.Array,
):
    del B_x
    B, S, D = A_x.shape
    _, H, Dh = A_Wq.shape
    M = A_mem0.shape[1]
    F = B_w3.shape[1]
    assert B == 1 and Dh == LANE
    kernel, scratch = _make_kernel(S, D, H, M, int(A_seg_len), F)
    hbm = pl.BlockSpec(memory_space=pl.ANY)
    vmem = pl.BlockSpec(memory_space=pltpu.VMEM)
    out = pl.pallas_call(
        kernel,
        in_specs=[hbm, vmem, hbm, hbm, hbm, hbm, hbm, hbm, hbm, hbm, vmem, hbm],
        out_specs=hbm,
        out_shape=jax.ShapeDtypeStruct((S, D), A_x.dtype),
        scratch_shapes=scratch,
        compiler_params=pltpu.CompilerParams(vmem_limit_bytes=127 * 1024 * 1024),
    )(A_x.reshape(S, D), A_mem0.reshape(M, D), A_Wq, A_Wk, A_Wv, A_Wo.reshape(H * Dh, D),
      B_w1, B_w2, B_w3, B_w4, c, w_mod)
    return out.reshape(B, S, D)
```

```python
import contextlib
import functools

import jax
import jax.numpy as jnp
import numpy as np
import jax.experimental.pallas as pl
import jax.experimental.pallas.tpu as pltpu

F32 = jnp.float32
BF16 = jnp.bfloat16
U32 = jnp.uint32
LANE = 128
CFG = dict(qk=2, v=3, pv=5, post=0, rb=128, fl=2, tie=1, prof=0)


def _scope(n):
    return jax.named_scope(n) if CFG['prof'] else contextlib.nullcontext()


def _loop(name, n, body):
    with _scope(name):
        jax.lax.fori_loop(0, n, body, 0)


def _dot(a, b):
    return jax.lax.dot_general(a, b, (((1,), (0,)), ((), ())), preferred_element_type=F32)


def _dot_nt(a, b):
    return jax.lax.dot_general(a, b, (((1,), (1,)), ((), ())), preferred_element_type=F32)


def _bf(w):
    return pltpu.bitcast(w, BF16)


def _pk(x):
    return pltpu.bitcast(x.astype(BF16), U32)


def _ln(x):
    m = jnp.mean(x, axis=-1, keepdims=True)
    xc = x - m
    v = jnp.mean(xc * xc, axis=-1, keepdims=True)
    return xc * jax.lax.rsqrt(v + 1e-5)


def _gelu(x):
    return jax.nn.gelu(x, approximate=True)


def _make_kernel(S, D, H, M, SEG, F):
    NSEG = S // SEG
    R = SEG - M
    P = S - R * NSEG
    RING = 576
    OFF = RING - P
    L = SEG + M
    HC = 16
    NCD = D // LANE
    BM = 512
    FC = 512
    PAD = 32
    LAG_QK, LAG_V, LAG_PV = CFG['qk'], CFG['v'], CFG['pv']
    scale = float(LANE) ** -0.5

    NHC = H // HC
    NCH = 3 * NHC
    NQ = 4
    DQ = D // NQ
    NST = 2
    MP = 512

    def kernel(x_hbm, mem0_ref, wq_hbm, wk_hbm, wv_hbm, wo_hbm, w1_hbm, w2_hbm, w3_hbm, w4_hbm, c_ref, wmod_hbm,
               out_hbm,
               x_s, h_s, h0_s, wo_s, w1_s, w2_s, w3_s, w4_s, wmod_s, ring_s, mod_s, modb_s, lhs_s, o_s, a_s,
               g_s, acc_s, ln_s, ob_s, z_s, t_s, sems, wsems, *rest):
        wqkv_s, stage_s = rest[:NCH], rest[NCH:]
        sem_i = iter(range(64))

        def copy(src, dst):
            return pltpu.make_async_copy(src, dst, sems.at[next(sem_i)])

        def cp_w(ch, k):
            rows = pl.ds(pl.multiple_of(k * DQ, DQ), DQ)
            src = (wq_hbm, wk_hbm, wv_hbm)[ch // NHC].at[rows, pl.ds((ch % NHC) * HC, HC), :]
            return pltpu.make_async_copy(src, stage_s[ch % NST].at[rows].bitcast(BF16), wsems.at[ch * NQ + k])

        cp_mod = [copy(wmod_hbm.at[:, pl.ds(MP * j, MP)], wmod_s.at[j].bitcast(BF16)) for j in range(6 * D // MP)]
        NMA = 2 * D // MP
        cp_x0 = copy(x_hbm.at[pl.ds(0, P)], x_s.at[pl.ds(PAD, P)])
        cp_x1 = copy(x_hbm.at[pl.ds(P, S - P)], x_s.at[pl.ds(PAD + P, S - P)])
        cp_wo = [copy(wo_hbm, wo_s.bitcast(BF16))]
        cp_w1 = [copy(w1_hbm, w1_s.bitcast(BF16))]
        cp_w2 = copy(w2_hbm, w2_s.bitcast(BF16))
        cp_w3 = [copy(w3_hbm.at[:, pl.ds(j * FC, FC)], w3_s.at[j].bitcast(BF16)) for j in range(F // FC)]
        cp_w4 = copy(w4_hbm, w4_s.bitcast(BF16))

        for k in range(NQ):
            cp_w(0, k).start()
        cp_x0.start()
        for cp in cp_mod[:NMA]:
            cp.start()
        for k in range(NQ):
            cp_w(1, k).start()

        cv = jnp.broadcast_to(c_ref[...].astype(F32), (8, D))
        sc = cv * jax.nn.sigmoid(cv)

        def mod(i):
            if i < 2:
                return mod_s[pl.ds(0, 1), pl.ds(i * D, D)]
            n = D // MP
            return jnp.concatenate([modb_s[(i - 2) * n + j, pl.ds(0, 1), :] for j in range(n)], axis=1)

        x_s[pl.ds(0, PAD), :] = jnp.zeros((PAD, D), BF16)
        a_s[...] = jnp.zeros(a_s.shape, F32)
        z_s[...] = jnp.zeros(z_s.shape, U32)
        g_s[pl.ds(PAD + S, 8), :] = jnp.zeros((8, D), F32)

        def relayout(ch, k, us, tie=None):
            for u in us:
                d0 = pl.multiple_of(k * DQ + u * 16, 16)
                v = stage_s[ch % NST][pl.ds(d0, 16), :, :]
                if tie is not None and CFG['tie']:
                    v = v | tie[None]
                v = v.reshape(8, 2, HC // 2, LANE)
                a, b = v[:, 0], v[:, 1]
                lo = (a & 0xFFFF) | (b << 16)
                hi = (a >> 16) | (b & np.uint32(0xFFFF0000))
                t0 = (u % 4) * 144
                for q in range(8):
                    t_s[pl.ds(t0 + q * 9, 8), :] = lo[q]
                    t_s[pl.ds(t0 + 72 + q * 9, 8), :] = hi[q]
                rows = pl.ds(pl.multiple_of(k * (DQ // 2) + u * 8, 8), 8)
                for j in range(HC // 2):
                    wqkv_s[ch][2 * j, rows, :] = t_s[pl.ds(t0 + j, 8, stride=9), :]
                    wqkv_s[ch][2 * j + 1, rows, :] = t_s[pl.ds(t0 + 72 + j, 8, stride=9), :]

        def first_chunk(k, carry):
            cp_w(0, k).wait()
            relayout(0, k, range(DQ // 16))
            return carry
        _loop('first', NQ, first_chunk)
        if NST < NCH:
            for k in range(NQ):
                cp_w(NST, k).start()
        cp_x1.start()

        cp_x0.wait()
        n0_s = acc_s
        def ln0(i, carry):
            r = pl.multiple_of(i * 128, 128)
            n0_s[pl.ds(r, 128), :] = _ln(x_s[pl.ds(pl.multiple_of(PAD + r, 32), 128), :].astype(F32))
            return carry
        _loop('ln0', P // 128, ln0)
        for j in range(NMA):
            cp_mod[j].wait()
            mod_s[:, pl.ds(MP * j, MP)] = _dot(sc, _bf(wmod_s[j]))
        h0_s[...] = _pk(n0_s[...] * (1.0 + mod(1)) + mod(0))

        for ch in range(NCH):
            last = ch == NCH - 1
            if last:
                cp_x1.wait()
                for cp in cp_mod[NMA:]:
                    cp.wait()

            def bulk(k, carry, ch=ch, last=last):
                if not last:
                    cp_w(ch + 1, k).wait()
                nh = HC // NQ
                nm = (len(cp_mod) - NMA) // NQ
                nr = (S - P) // NQ
                RB = CFG['rb']
                nb = P // RB
                for u in range(nh):
                    j = k * nh + u
                    for t in range(nb):
                        y = _dot(_bf(h0_s[pl.ds(t * RB // 2, RB // 2), :]), _bf(wqkv_s[ch][j]))
                        ring_s[ch * HC + j, pl.ds(OFF + t * RB, RB), :] = y.astype(BF16)
                        piece = u * nb + t
                        tie = pltpu.bitcast(y[:8], U32) & z_s[...]
                        if not last:
                            n = DQ // 16 // (nh * nb)
                            relayout(ch + 1, k, range(piece * n, piece * n + n), tie)
                        else:
                            if piece < nr // 32:
                                r = pl.multiple_of(PAD + P + k * nr + piece * 32, 32)
                                xv = pltpu.bitcast(x_s[pl.ds(r, 32), :], U32) | jnp.tile(tie, (2, NCD))
                                xv = pltpu.bitcast(xv, BF16).astype(F32)
                                h_s[pl.ds(r, 32), :] = (_ln(xv) * (1.0 + mod(1)) + mod(0)).astype(BF16)
                            if piece < nm * MP // LANE:
                                a, b = divmod(piece, MP // LANE)
                                cols = pl.ds(b * LANE, LANE)
                                modb_s[k * nm + a, :, cols] = _dot(sc, _bf(wmod_s[NMA + k * nm + a, :, cols]))
                return carry
            _loop(f'bulk{ch}', NQ, bulk)
            if ch + 1 + NST < NCH:
                for k in range(NQ):
                    cp_w(ch + 1 + NST, k).start()
            if ch == 0:
                for cp in cp_mod[NMA:NMA + 4]:
                    cp.start()
            if ch == 1:
                for cp in cp_mod[NMA + 4:]:
                    cp.start()
            if ch == 2:
                for cp in cp_wo + cp_w1 + [cp_w2] + cp_w3 + [cp_w4]:
                    cp.start()

        for cp in cp_wo + cp_w1:
            cp.wait()

        lhs_s[...] = mem0_ref[...].astype(F32)

        row = jax.lax.broadcasted_iota(jnp.int32, (L, L), 0)
        col = jax.lax.broadcasted_iota(jnp.int32, (L, L), 1)

        def post_attention(r):
            x1 = (x_s[pl.ds(r, SEG), :].astype(F32) + mod(2) * a_s[...]).astype(BF16)
            x_s[pl.ds(r, SEG), :] = x1
            h2 = (_ln(x1.astype(F32)) * (1.0 + mod(4)) + mod(3)).astype(BF16)
            h_s[pl.ds(r, SEG), :] = h2
            n2 = _ln(h2.astype(F32)).astype(BF16)
            return n2

        def w1_stage(n2, r):
            for j in range(NCD):
                g_s[pl.ds(r, SEG), pl.ds(j * LANE, LANE)] = _gelu(_dot(n2, _bf(w1_s[:, pl.ds(j * LANE, LANE)])))

        def step(s, carry):
            mask = (row >= SEG) | (col >= SEG) | (row >= col)
            wpos = pl.multiple_of(jax.lax.rem(s * R, RING), 8)
            rpos = pl.multiple_of(jax.lax.rem(s * SEG + OFF, RING), SEG)
            tok = h_s[pl.ds(pl.multiple_of(PAD + P + s * R, 8), R), :].astype(F32)
            lhs = jnp.concatenate([tok, lhs_s[...]], axis=0).astype(BF16)
            prev = pl.multiple_of(PAD + (s - 1) * SEG, SEG)
            n2 = post_attention(prev)

            def proj(j):
                y = _dot(lhs, _bf(wqkv_s[j // HC][j % HC]))
                ring_s[j, pl.ds(wpos, R), :] = y[:R].astype(BF16)
                return y[R:]

            def full(j, m):
                return jnp.concatenate([ring_s[j, pl.ds(rpos, SEG), :].astype(F32), m], axis=0)

            qs, ks, vs, pr = {}, {}, {}, {}
            for i in range(H + LAG_PV):
                if i < H:
                    qm = proj(i)
                if 0 <= i - LAG_QK < H:
                    hq = i - LAG_QK
                    sco = jnp.where(mask, _dot_nt(qs.pop(hq), ks.pop(hq)) * scale, -1e9)
                    e = jnp.exp(sco - jnp.max(sco, axis=-1, keepdims=True))
                    pr[hq] = e if CFG['post'] else e / jnp.sum(e, axis=-1, keepdims=True)
                if i < H:
                    km = proj(H + i)
                    qs[i] = full(i, qm)
                    ks[i] = full(H + i, km)
                if 0 <= i - LAG_V < H:
                    hv = i - LAG_V
                    vs[hv] = full(2 * H + hv, proj(2 * H + hv))
                if i == H + LAG_V:
                    w1_stage(n2, prev)
                if 0 <= i - LAG_PV < H:
                    hp = i - LAG_PV
                    e = pr.pop(hp)
                    o = _dot(e, vs.pop(hp))
                    if CFG['post']:
                        o = o * (1.0 / jnp.sum(e, axis=-1, keepdims=True))
                    o_s[:, pl.ds(hp * LANE, LANE)] = o
            for j in range(NCD):
                y = _dot(o_s[...], _bf(wo_s[:, pl.ds(j * LANE, LANE)]))
                a_s[:, pl.ds(j * LANE, LANE)] = y[:SEG]
                lhs_s[:, pl.ds(j * LANE, LANE)] = y[SEG:]
            return carry

        _loop('steps', NSEG, step)
        last = PAD + S - SEG
        w1_stage(post_attention(last), last)
        g_s[pl.ds(PAD - 8, 8), :] = jnp.zeros((8, D), F32)

        for cp in [cp_w2] + cp_w3 + [cp_w4]:
            cp.wait()

        osem = next(sem_i)

        def out_copy(b):
            return pltpu.make_async_copy(ob_s, out_hbm.at[pl.ds(pl.multiple_of(b * BM, BM), BM)], sems.at[osem])

        Q = D // 4

        def block(b, carry):
            r = pl.multiple_of(PAD + b * BM, 32)
            parts = []
            for gi, sh in enumerate((-1, 1, -2, 2)):
                gv = g_s[pl.ds(pl.multiple_of(r - 8, 8), BM + 16), pl.ds(gi * Q, Q)]
                parts.append(gv[8 + sh:8 + sh + BM].astype(BF16))
            y1 = h_s[pl.ds(r, BM), :].astype(F32) + _dot(jnp.concatenate(parts, axis=1), _bf(w2_s[...]))
            acc_s[...] = y1
            ln_s[...] = _pk(_ln(y1))

            def mlp(f, carry):
                u = _gelu(_dot(_bf(ln_s[...]), _bf(w3_s[f]))).astype(BF16)
                acc_s[...] += _dot(u, _bf(w4_s[pl.ds(pl.multiple_of(f * (FC // 2), FC // 2), FC // 2), :]))
                return carry
            _loop('mlp', F // FC, mlp)

            @pl.when(b > 0)
            def _():
                out_copy(b - 1).wait()
            ob_s[...] = (x_s[pl.ds(r, BM), :].astype(F32) + mod(5) * acc_s[...]).astype(BF16)
            out_copy(b).start()
            return carry

        _loop('B', S // BM, block)
        out_copy(S // BM - 1).wait()

    scratch = [
        pltpu.VMEM((PAD + S, D), BF16),
        pltpu.VMEM((PAD + S, D), BF16),
        pltpu.VMEM((P // 2, D), U32),
        pltpu.VMEM((H * LANE // 2, D), U32),
        pltpu.VMEM((D // 2, D), U32),
        pltpu.VMEM((D // 2, D), U32),
        pltpu.VMEM((F // FC, D // 2, FC), U32),
        pltpu.VMEM((F // 2, D), U32),
        pltpu.VMEM((6 * D // MP, D // 2, MP), U32),
        pltpu.VMEM((3 * H, RING, LANE), BF16),
        pltpu.VMEM((8, 2 * D), F32),
        pltpu.VMEM((4 * D // MP, 8, MP), F32),
        pltpu.VMEM((M, D), F32),
        pltpu.VMEM((L, H * LANE), F32),
        pltpu.VMEM((SEG, D), F32),
        pltpu.VMEM((PAD + S + 8, D), F32),
        pltpu.VMEM((BM, D), F32),
        pltpu.VMEM((BM // 2, D), U32),
        pltpu.VMEM((BM, D), BF16),
        pltpu.VMEM((8, LANE), U32),
        pltpu.VMEM((592, LANE), U32),
        pltpu.SemaphoreType.DMA((64,)),
        pltpu.SemaphoreType.DMA((NCH * NQ,)),
    ]
    scratch += [pltpu.VMEM((HC, D // 2, LANE), U32)] * NCH + [pltpu.VMEM((D, HC // 2, LANE), U32)] * NST
    return kernel, scratch


@functools.partial(jax.jit, static_argnames=("A_seg_len",))
def pallas_adaLN_cond__memory_aug_recurrent_mem_tr__mixer_s_mlp__prompt_kernel(
    A_x: jax.Array,
    A_mem0: jax.Array,
    A_Wq: jax.Array,
    A_Wk: jax.Array,
    A_Wv: jax.Array,
    A_Wo: jax.Array,
    A_seg_len: int,
    B_x: jax.Array,
    B_w1: jax.Array,
    B_w2: jax.Array,
    B_w3: jax.Array,
    B_w4: jax.Array,
    c: jax.Array,
    w_mod: jax.Array,
):
    del B_x
    B, S, D = A_x.shape
    _, H, Dh = A_Wq.shape
    M = A_mem0.shape[1]
    F = B_w3.shape[1]
    assert B == 1 and Dh == LANE
    kernel, scratch = _make_kernel(S, D, H, M, int(A_seg_len), F)
    hbm = pl.BlockSpec(memory_space=pl.ANY)
    vmem = pl.BlockSpec(memory_space=pltpu.VMEM)
    out = pl.pallas_call(
        kernel,
        in_specs=[hbm, vmem, hbm, hbm, hbm, hbm, hbm, hbm, hbm, hbm, vmem, hbm],
        out_specs=hbm,
        out_shape=jax.ShapeDtypeStruct((S, D), A_x.dtype),
        scratch_shapes=scratch,
        compiler_params=pltpu.CompilerParams(vmem_limit_bytes=127 * 1024 * 1024, flags={0: None, 1: {'XLA_TPU_FORCE_LP_LLO_SCHEDULER': True}, 2: {'XLA_TPU_EVENLY_DISTRIBUTE_CRITICAL_NODES': True}}[CFG['fl']]),
    )(A_x.reshape(S, D), A_mem0.reshape(M, D), A_Wq, A_Wk, A_Wv, A_Wo.reshape(H * Dh, D),
      B_w1, B_w2, B_w3, B_w4, c, w_mod)
    return out.reshape(B, S, D)
```

```python
import contextlib
import functools

import jax
import jax.numpy as jnp
import numpy as np
import jax.experimental.pallas as pl
import jax.experimental.pallas.tpu as pltpu

F32 = jnp.float32
BF16 = jnp.bfloat16
U32 = jnp.uint32
LANE = 128
CFG = dict(qk=2, v=3, pv=5, post=0, rb=128, fl=2, tie=1, prof=0, w1=8, rb1=128, rb2=128, bm=1024)


def _scope(n):
    return jax.named_scope(n) if CFG['prof'] else contextlib.nullcontext()


def _loop(name, n, body):
    with _scope(name):
        jax.lax.fori_loop(0, n, body, 0)


def _dot(a, b):
    return jax.lax.dot_general(a, b, (((1,), (0,)), ((), ())), preferred_element_type=F32)


def _dot_nt(a, b):
    return jax.lax.dot_general(a, b, (((1,), (1,)), ((), ())), preferred_element_type=F32)


def _bf(w):
    return pltpu.bitcast(w, BF16)


def _pk(x):
    return pltpu.bitcast(x.astype(BF16), U32)


def _ln(x):
    m = jnp.mean(x, axis=-1, keepdims=True)
    xc = x - m
    v = jnp.mean(xc * xc, axis=-1, keepdims=True)
    return xc * jax.lax.rsqrt(v + 1e-5)


def _gelu(x):
    return jax.nn.gelu(x, approximate=True)


def _strassen_lhs(a11, a12, a21, a22):
    return a11 + a22, a21 + a22, a11, a22, a11 + a12, a21 - a11, a12 - a22


def _strassen(prod):
    m2 = prod(1)
    m5 = prod(4)
    m4 = prod(3)
    c21 = m2 + m4
    c11 = m4 - m5
    m3 = prod(2)
    c12 = m3 + m5
    c22 = m3 - m2
    m1 = prod(0)
    c11 = c11 + m1
    c22 = c22 + m1
    c11 = c11 + prod(6)
    c22 = c22 + prod(5)
    return c11, c12, c21, c22


def _make_kernel(S, D, H, M, SEG, F):
    NSEG = S // SEG
    R = SEG - M
    P = S - R * NSEG
    RING = 576
    OFF = RING - P
    L = SEG + M
    HC = 16
    NCD = D // LANE
    PAD = 2 * SEG
    G0 = 4 * SEG
    LAG_QK, LAG_V, LAG_PV = CFG['qk'], CFG['v'], CFG['pv']
    scale = float(LANE) ** -0.5

    NHC = H // HC
    NCH = 3 * NHC
    NQ = 4
    DQ = D // NQ
    NST = 2
    MP = 512

    def kernel(x_hbm, mem0_ref, wq_hbm, wk_hbm, wv_hbm, wo_hbm, w1_hbm, w2_hbm, w3_hbm, w4_hbm, c_ref, wmod_hbm,
               out_hbm,
               x_s, h_s, h0_s, wo_s, w1_s, w2_s, w3_s, w4_s, wmod_s, ring_s, mod_s, modb_s, lhs_s, o_s, a_s,
               g_s, n0_s, ws_s, u7_s, gb_s, ob_s, z_s, t_s, sems, wsems, *rest):
        wqkv_s, stage_s = rest[:NCH], rest[NCH:]
        sem_i = iter(range(64))

        def copy(src, dst):
            return pltpu.make_async_copy(src, dst, sems.at[next(sem_i)])

        def cp_w(ch, k):
            rows = pl.ds(pl.multiple_of(k * DQ, DQ), DQ)
            src = (wq_hbm, wk_hbm, wv_hbm)[ch // NHC].at[rows, pl.ds((ch % NHC) * HC, HC), :]
            return pltpu.make_async_copy(src, stage_s[ch % NST].at[rows].bitcast(BF16), wsems.at[ch * NQ + k])

        cp_mod = [copy(wmod_hbm.at[:, pl.ds(MP * j, MP)], wmod_s.at[j].bitcast(BF16)) for j in range(6 * D // MP)]
        NMA = 2 * D // MP
        cp_x0 = copy(x_hbm.at[pl.ds(0, P)], x_s.at[pl.ds(PAD, P)])
        cp_x1 = copy(x_hbm.at[pl.ds(P, S - P)], x_s.at[pl.ds(PAD + P, S - P)])
        cp_wo = [copy(wo_hbm, wo_s.bitcast(BF16))]
        cp_w1 = [copy(w1_hbm, w1_s.bitcast(BF16))]
        cp_w2 = copy(w2_hbm, w2_s.bitcast(BF16))
        cp_w3 = [copy(w3_hbm.at[:, pl.ds(j * LANE, LANE)], w3_s.at[j].bitcast(BF16)) for j in range(F // LANE)]
        cp_w4 = [copy(w4_hbm.at[:, pl.ds(j * LANE, LANE)], w4_s.at[j].bitcast(BF16)) for j in range(NCD)]

        for k in range(NQ):
            cp_w(0, k).start()
        cp_x0.start()
        for cp in cp_mod[:NMA]:
            cp.start()
        for k in range(NQ):
            cp_w(1, k).start()

        cv = jnp.broadcast_to(c_ref[...].astype(F32), (8, D))
        sc = cv * jax.nn.sigmoid(cv)

        def mod(i):
            if i < 2:
                return mod_s[pl.ds(0, 1), pl.ds(i * D, D)]
            n = D // MP
            return jnp.concatenate([modb_s[(i - 2) * n + j, pl.ds(0, 1), :] for j in range(n)], axis=1)

        x_s[pl.ds(0, PAD), :] = jnp.zeros((PAD, D), BF16)
        a_s[...] = jnp.zeros(a_s.shape, F32)
        z_s[...] = jnp.zeros(z_s.shape, U32)
        h_s[pl.ds(0, PAD), :] = jnp.zeros((PAD, D), BF16)
        g_s[pl.ds(0, G0), :] = jnp.zeros((G0, D), F32)
        g_s[pl.ds(G0 + S, 8), :] = jnp.zeros((8, D), F32)

        def relayout(ch, k, us, tie=None):
            for u in us:
                d0 = pl.multiple_of(k * DQ + u * 16, 16)
                v = stage_s[ch % NST][pl.ds(d0, 16), :, :]
                if tie is not None and CFG['tie']:
                    v = v | tie[None]
                v = v.reshape(8, 2, HC // 2, LANE)
                a, b = v[:, 0], v[:, 1]
                lo = (a & 0xFFFF) | (b << 16)
                hi = (a >> 16) | (b & np.uint32(0xFFFF0000))
                t0 = (u % 4) * 144
                for q in range(8):
                    t_s[pl.ds(t0 + q * 9, 8), :] = lo[q]
                    t_s[pl.ds(t0 + 72 + q * 9, 8), :] = hi[q]
                rows = pl.ds(pl.multiple_of(k * (DQ // 2) + u * 8, 8), 8)
                for j in range(HC // 2):
                    wqkv_s[ch][2 * j, rows, :] = t_s[pl.ds(t0 + j, 8, stride=9), :]
                    wqkv_s[ch][2 * j + 1, rows, :] = t_s[pl.ds(t0 + 72 + j, 8, stride=9), :]

        def first_chunk(k, carry):
            cp_w(0, k).wait()
            relayout(0, k, range(DQ // 16))
            return carry
        _loop('first', NQ, first_chunk)
        if NST < NCH:
            for k in range(NQ):
                cp_w(NST, k).start()
        cp_x1.start()

        cp_x0.wait()
        def ln0(i, carry):
            r = pl.multiple_of(i * 128, 128)
            n0_s[pl.ds(r, 128), :] = _ln(x_s[pl.ds(pl.multiple_of(PAD + r, 32), 128), :].astype(F32))
            return carry
        _loop('ln0', P // 128, ln0)
        for j in range(NMA):
            cp_mod[j].wait()
            mod_s[:, pl.ds(MP * j, MP)] = _dot(sc, _bf(wmod_s[j]))
        h0_s[...] = _pk(n0_s[...] * (1.0 + mod(1)) + mod(0))

        for ch in range(NCH):
            last = ch == NCH - 1
            if last:
                cp_x1.wait()
                for cp in cp_mod[NMA:]:
                    cp.wait()

            def bulk(k, carry, ch=ch, last=last):
                if not last:
                    cp_w(ch + 1, k).wait()
                nh = HC // NQ
                nm = (len(cp_mod) - NMA) // NQ
                nr = (S - P) // NQ
                RB = CFG['rb']
                nb = P // RB
                for u in range(nh):
                    j = k * nh + u
                    for t in range(nb):
                        y = _dot(_bf(h0_s[pl.ds(t * RB // 2, RB // 2), :]), _bf(wqkv_s[ch][j]))
                        ring_s[ch * HC + j, pl.ds(OFF + t * RB, RB), :] = y.astype(BF16)
                        piece = u * nb + t
                        tie = pltpu.bitcast(y[:8], U32) & z_s[...]
                        if not last:
                            n = DQ // 16 // (nh * nb)
                            relayout(ch + 1, k, range(piece * n, piece * n + n), tie)
                        else:
                            if piece < nr // 32:
                                r = pl.multiple_of(PAD + P + k * nr + piece * 32, 32)
                                xv = pltpu.bitcast(x_s[pl.ds(r, 32), :], U32) | jnp.tile(tie, (2, NCD))
                                xv = pltpu.bitcast(xv, BF16).astype(F32)
                                h_s[pl.ds(r, 32), :] = (_ln(xv) * (1.0 + mod(1)) + mod(0)).astype(BF16)
                            if piece < nm * MP // LANE:
                                a, b = divmod(piece, MP // LANE)
                                cols = pl.ds(b * LANE, LANE)
                                modb_s[k * nm + a, :, cols] = _dot(sc, _bf(wmod_s[NMA + k * nm + a, :, cols]))
                return carry
            _loop(f'bulk{ch}', NQ, bulk)
            if ch + 1 + NST < NCH:
                for k in range(NQ):
                    cp_w(ch + 1 + NST, k).start()
            if ch == 0:
                for cp in cp_mod[NMA:NMA + 4]:
                    cp.start()
            if ch == 1:
                for cp in cp_mod[NMA + 4:]:
                    cp.start()
            if ch == 2:
                for cp in cp_wo + cp_w1 + [cp_w2]:
                    cp.start()

        for cp in cp_wo + cp_w1 + [cp_w2]:
            cp.wait()
        for cp in cp_w3 + cp_w4:
            cp.start()

        lhs_s[...] = mem0_ref[...].astype(F32)

        row = jax.lax.broadcasted_iota(jnp.int32, (L, L), 0)
        col = jax.lax.broadcasted_iota(jnp.int32, (L, L), 1)

        def seg_rows(base, j):
            r = base + j * SEG
            return r if isinstance(r, int) else pl.multiple_of(r, SEG)

        def post_attention(j):
            r = seg_rows(PAD, j)
            x1 = (x_s[pl.ds(r, SEG), :].astype(F32) + mod(2) * a_s[...]).astype(BF16)
            x_s[pl.ds(r, SEG), :] = x1
            h2 = (_ln(x1.astype(F32)) * (1.0 + mod(4)) + mod(3)).astype(BF16)
            h_s[pl.ds(r, SEG), :] = h2
            return _ln(h2.astype(F32)).astype(BF16)

        def w1_stage(n2, j):
            r = seg_rows(G0, j)
            for n in range(NCD):
                g = _gelu(_dot(n2, _bf(w1_s[:, pl.ds(n * LANE, LANE)])))
                g_s[pl.ds(r, SEG), pl.ds(n * LANE, LANE)] = jnp.where(j >= 0, g, 0.0)

        def w2_stage(j):
            r = seg_rows(G0, j)
            parts = []
            for gi, sh in enumerate((-1, 1, -2, 2)):
                gv = g_s[pl.ds(r - 8, SEG + 16), pl.ds(gi * (D // 4), D // 4)]
                parts.append(gv[8 + sh:8 + sh + SEG].astype(BF16))
            gs = jnp.concatenate(parts, axis=1)
            rp = seg_rows(PAD, j)
            y = h_s[pl.ds(rp, SEG), :].astype(F32) + _dot(gs, _bf(w2_s[...]))
            g_s[pl.ds(seg_rows(G0 - 2 * SEG, j), SEG), :] = x_s[pl.ds(rp, SEG), :].astype(F32) + mod(5) * y
            n = _ln(y)
            hs, hd = SEG // 2, D // 2
            ro = jnp.maximum(j, 0) * (SEG // 4)
            ro = ro if isinstance(j, int) else pl.multiple_of(ro, SEG // 4)
            for i, op in enumerate(_strassen_lhs(n[:hs, :hd], n[:hs, hd:], n[hs:, :hd], n[hs:, hd:])):
                wmod_s[i, pl.ds(ro, SEG // 4), :] = _pk(op)

        def step(s, carry):
            mask = (row >= SEG) | (col >= SEG) | (row >= col)
            wpos = pl.multiple_of(jax.lax.rem(s * R, RING), 8)
            rpos = pl.multiple_of(jax.lax.rem(s * SEG + OFF, RING), SEG)
            tok = h_s[pl.ds(pl.multiple_of(PAD + P + s * R, 8), R), :].astype(F32)
            lhs = jnp.concatenate([tok, lhs_s[...]], axis=0).astype(BF16)
            n2 = post_attention(s - 1)

            def proj(j):
                y = _dot(lhs, _bf(wqkv_s[j // HC][j % HC]))
                ring_s[j, pl.ds(wpos, R), :] = y[:R].astype(BF16)
                return y[R:]

            def full(j, m):
                return jnp.concatenate([ring_s[j, pl.ds(rpos, SEG), :].astype(F32), m], axis=0)

            qs, ks, vs, pr = {}, {}, {}, {}
            for i in range(H + LAG_PV):
                if i < H:
                    qm = proj(i)
                if 0 <= i - LAG_QK < H:
                    hq = i - LAG_QK
                    sco = jnp.where(mask, _dot_nt(qs.pop(hq), ks.pop(hq)) * scale, -1e9)
                    e = jnp.exp(sco - jnp.max(sco, axis=-1, keepdims=True))
                    pr[hq] = e if CFG['post'] else e / jnp.sum(e, axis=-1, keepdims=True)
                if i < H:
                    km = proj(H + i)
                    qs[i] = full(i, qm)
                    ks[i] = full(H + i, km)
                if 0 <= i - LAG_V < H:
                    hv = i - LAG_V
                    vs[hv] = full(2 * H + hv, proj(2 * H + hv))
                if i == CFG['w1']:
                    w1_stage(n2, s - 1)
                if i == H + LAG_V:
                    w2_stage(s - 2)
                if 0 <= i - LAG_PV < H:
                    hp = i - LAG_PV
                    e = pr.pop(hp)
                    o = _dot(e, vs.pop(hp))
                    if CFG['post']:
                        o = o * (1.0 / jnp.sum(e, axis=-1, keepdims=True))
                    o_s[:, pl.ds(hp * LANE, LANE)] = o
            for j in range(NCD):
                y = _dot(o_s[...], _bf(wo_s[:, pl.ds(j * LANE, LANE)]))
                a_s[:, pl.ds(j * LANE, LANE)] = y[:SEG]
                lhs_s[:, pl.ds(j * LANE, LANE)] = y[SEG:]
            return carry

        _loop('steps', NSEG, step)
        w1_stage(post_attention(NSEG - 1), NSEG - 1)
        w2_stage(NSEG - 2)
        w2_stage(NSEG - 1)

        for cp in cp_w3 + cp_w4:
            cp.wait()

        NT = F // 2 // LANE
        HS = S // 2

        def u_op(i, t):
            if i < NCH:
                return wqkv_s[i].at[t]
            return u7_s.at[t]

        def rhs_sums(w, n1, n2, kh):
            b11, b12 = w.at[n1, pl.ds(0, kh)], w.at[n2, pl.ds(0, kh)]
            b21, b22 = w.at[n1, pl.ds(kh, kh)], w.at[n2, pl.ds(kh, kh)]
            for r in range(0, kh, 32):
                rows = pl.ds(r, 32)
                v11, v12, v21, v22 = (_bf(b[rows, :]).astype(F32) for b in (b11, b12, b21, b22))
                for i, v in enumerate((v11 + v22, v12 - v22, v21 - v11, v11 + v12, v21 + v22)):
                    ws_s[i, rows, :] = _pk(v)
            sm = [ws_s.at[i, pl.ds(0, kh)] for i in range(5)]
            return [sm[0], b11, sm[1], sm[2], b22, sm[3], sm[4]]

        def mlp1(t, carry):
            b = rhs_sums(w3_s, t, NT + t, D // 4)
            RB = CFG['rb1']
            for r in range(0, HS, RB):
                rows = pl.ds(r // 2, RB // 2)
                c = _strassen(lambda i: _dot(_bf(wmod_s[i, rows, :]), _bf(b[i][...])))
                for i, op in enumerate(_strassen_lhs(*map(_gelu, c))):
                    u_op(i, t)[rows, :] = _pk(op)
            return carry
        _loop('mlp1', NT, mlp1)

        NH = NCD // 2
        BM = CFG['bm']
        osem = next(sem_i)
        next(sem_i)

        def out_copy(it, half):
            rows = pl.ds(pl.multiple_of((it // NH) * BM, BM), BM)
            cols = pl.ds(pl.multiple_of((it % NH + half * NH) * LANE, LANE), LANE)
            return pltpu.make_async_copy(ob_s.at[half], out_hbm.at[rows, cols], sems.at[osem + half])

        def mlp2(it, carry):
            @pl.when(it > 0)
            def _():
                out_copy(it - 1, 0).wait()
                out_copy(it - 1, 1).wait()
            blk, n = it // NH, it % NH
            b = rhs_sums(w4_s, n, NH + n, F // 4)
            RB = CFG['rb2']
            for r in range(0, BM // 2, RB):
                rows = pl.ds(pl.multiple_of(blk * (BM // 4) + r // 2, RB // 2), RB // 2)

                def prod(i):
                    lhs = jnp.concatenate([_bf(u_op(i, t)[rows, :]) for t in range(NT)], axis=1)
                    return _dot(lhs, _bf(b[i][...]))
                c11, c12, c21, c22 = _strassen(prod)
                for half, (ct, cb) in enumerate(((c11, c21), (c12, c22))):
                    cols = pl.ds(pl.multiple_of((n + half * NH) * LANE, LANE), LANE)
                    hs = SEG // 2
                    y = jnp.concatenate([v[q:q + hs] for q in range(0, RB, hs) for v in (ct, cb)], axis=0)
                    base = g_s[pl.ds(pl.multiple_of(G0 - 2 * SEG + blk * BM + 2 * r, SEG), 2 * RB), cols]
                    ob_s[half, pl.ds(2 * r, 2 * RB), :] = (base + gb_s[n + half * NH, pl.ds(0, 1), :] * y).astype(BF16)
            out_copy(it, 0).start()
            out_copy(it, 1).start()
            return carry
        for n in range(NCD):
            gb_s[n] = jnp.broadcast_to(mod(5)[:, n * LANE:(n + 1) * LANE], (8, LANE))
        nit = (S // BM) * NH
        _loop('mlp2', nit, mlp2)
        out_copy(nit - 1, 0).wait()
        out_copy(nit - 1, 1).wait()

    scratch = [
        pltpu.VMEM((PAD + S, D), BF16),
        pltpu.VMEM((PAD + S, D), BF16),
        pltpu.VMEM((P // 2, D), U32),
        pltpu.VMEM((H * LANE // 2, D), U32),
        pltpu.VMEM((D // 2, D), U32),
        pltpu.VMEM((D // 2, D), U32),
        pltpu.VMEM((F // LANE, D // 2, LANE), U32),
        pltpu.VMEM((NCD, F // 2, LANE), U32),
        pltpu.VMEM((6 * D // MP, D // 2, MP), U32),
        pltpu.VMEM((3 * H, RING, LANE), BF16),
        pltpu.VMEM((8, 2 * D), F32),
        pltpu.VMEM((4 * D // MP, 8, MP), F32),
        pltpu.VMEM((M, D), F32),
        pltpu.VMEM((L, H * LANE), F32),
        pltpu.VMEM((SEG, D), F32),
        pltpu.VMEM((G0 + S + 8, D), F32),
        pltpu.VMEM((P, D), F32),
        pltpu.VMEM((5, F // 4, LANE), U32),
        pltpu.VMEM((F // 2 // LANE, S // 4, LANE), U32),
        pltpu.VMEM((NCD, 8, LANE), F32),
        pltpu.VMEM((2, CFG['bm'], LANE), BF16),
        pltpu.VMEM((8, LANE), U32),
        pltpu.VMEM((592, LANE), U32),
        pltpu.SemaphoreType.DMA((64,)),
        pltpu.SemaphoreType.DMA((NCH * NQ,)),
    ]
    scratch += [pltpu.VMEM((HC, D // 2, LANE), U32)] * NCH + [pltpu.VMEM((D, HC // 2, LANE), U32)] * NST
    return kernel, scratch


@functools.partial(jax.jit, static_argnames=("A_seg_len",))
def pallas_adaLN_cond__memory_aug_recurrent_mem_tr__mixer_s_mlp__prompt_kernel(
    A_x: jax.Array,
    A_mem0: jax.Array,
    A_Wq: jax.Array,
    A_Wk: jax.Array,
    A_Wv: jax.Array,
    A_Wo: jax.Array,
    A_seg_len: int,
    B_x: jax.Array,
    B_w1: jax.Array,
    B_w2: jax.Array,
    B_w3: jax.Array,
    B_w4: jax.Array,
    c: jax.Array,
    w_mod: jax.Array,
):
    del B_x
    B, S, D = A_x.shape
    _, H, Dh = A_Wq.shape
    M = A_mem0.shape[1]
    F = B_w3.shape[1]
    assert B == 1 and Dh == LANE
    kernel, scratch = _make_kernel(S, D, H, M, int(A_seg_len), F)
    hbm = pl.BlockSpec(memory_space=pl.ANY)
    vmem = pl.BlockSpec(memory_space=pltpu.VMEM)
    out = pl.pallas_call(
        kernel,
        in_specs=[hbm, vmem, hbm, hbm, hbm, hbm, hbm, hbm, hbm, hbm, vmem, hbm],
        out_specs=hbm,
        out_shape=jax.ShapeDtypeStruct((S, D), A_x.dtype),
        scratch_shapes=scratch,
        compiler_params=pltpu.CompilerParams(vmem_limit_bytes=127 * 1024 * 1024, flags={0: None, 1: {'XLA_TPU_FORCE_LP_LLO_SCHEDULER': True}, 2: {'XLA_TPU_EVENLY_DISTRIBUTE_CRITICAL_NODES': True}}[CFG['fl']]),
    )(A_x.reshape(S, D), A_mem0.reshape(M, D), A_Wq, A_Wk, A_Wv, A_Wo.reshape(H * Dh, D),
      B_w1, B_w2, B_w3, B_w4, c, w_mod)
    return out.reshape(B, S, D)
```

```python
import contextlib
import functools

import jax
import jax.numpy as jnp
import numpy as np
import jax.experimental.pallas as pl
import jax.experimental.pallas.tpu as pltpu

F32 = jnp.float32
BF16 = jnp.bfloat16
U32 = jnp.uint32
LANE = 128
CFG = dict(qk=2, v=3, pv=5, post=0, rb=128, fl=2, tie=1, prof=0, w1=8, rb1=128, rb2=512, bm=1024)


def _scope(n):
    return jax.named_scope(n) if CFG['prof'] else contextlib.nullcontext()


def _loop(name, n, body):
    with _scope(name):
        jax.lax.fori_loop(0, n, body, 0)


def _dot(a, b):
    return jax.lax.dot_general(a, b, (((1,), (0,)), ((), ())), preferred_element_type=F32)


def _dot_nt(a, b):
    return jax.lax.dot_general(a, b, (((1,), (1,)), ((), ())), preferred_element_type=F32)


def _bf(w):
    return pltpu.bitcast(w, BF16)


def _pk(x):
    return pltpu.bitcast(x.astype(BF16), U32)


def _ln(x):
    m = jnp.mean(x, axis=-1, keepdims=True)
    xc = x - m
    v = jnp.mean(xc * xc, axis=-1, keepdims=True)
    return xc * jax.lax.rsqrt(v + 1e-5)


def _gelu(x):
    return jax.nn.gelu(x, approximate=True)


def _strassen_lhs(a11, a12, a21, a22):
    return a11 + a22, a21 + a22, a11, a22, a11 + a12, a21 - a11, a12 - a22


def _strassen(prod):
    m2 = prod(1)
    m5 = prod(4)
    m4 = prod(3)
    c21 = m2 + m4
    c11 = m4 - m5
    m3 = prod(2)
    c12 = m3 + m5
    c22 = m3 - m2
    m1 = prod(0)
    c11 = c11 + m1
    c22 = c22 + m1
    c11 = c11 + prod(6)
    c22 = c22 + prod(5)
    return c11, c12, c21, c22


def _make_kernel(S, D, H, M, SEG, F):
    NSEG = S // SEG
    R = SEG - M
    P = S - R * NSEG
    RING = 576
    OFF = RING - P
    L = SEG + M
    HC = 16
    NCD = D // LANE
    PAD = 2 * SEG
    G0 = 4 * SEG
    LAG_QK, LAG_V, LAG_PV = CFG['qk'], CFG['v'], CFG['pv']
    scale = float(LANE) ** -0.5

    NHC = H // HC
    NCH = 3 * NHC
    NQ = 4
    DQ = D // NQ
    NST = 2
    MP = 512

    def kernel(x_hbm, mem0_ref, wq_hbm, wk_hbm, wv_hbm, wo_hbm, w1_hbm, w2_hbm, w3_hbm, w4_hbm, c_ref, wmod_hbm,
               out_hbm,
               x_s, h_s, h0_s, wo_s, w1_s, w2_s, w3_s, w4_s, wmod_s, ring_s, mod_s, modb_s, lhs_s, o_s, a_s,
               g_s, n0_s, ws_s, u7_s, gb_s, ob_s, z_s, t_s, sems, wsems, *rest):
        wqkv_s, stage_s = rest[:NCH], rest[NCH:]
        sem_i = iter(range(64))

        def copy(src, dst):
            return pltpu.make_async_copy(src, dst, sems.at[next(sem_i)])

        def cp_w(ch, k):
            rows = pl.ds(pl.multiple_of(k * DQ, DQ), DQ)
            src = (wq_hbm, wk_hbm, wv_hbm)[ch // NHC].at[rows, pl.ds((ch % NHC) * HC, HC), :]
            return pltpu.make_async_copy(src, stage_s[ch % NST].at[rows].bitcast(BF16), wsems.at[ch * NQ + k])

        cp_mod = [copy(wmod_hbm.at[:, pl.ds(MP * j, MP)], wmod_s.at[j].bitcast(BF16)) for j in range(6 * D // MP)]
        NMA = 2 * D // MP
        cp_x0 = copy(x_hbm.at[pl.ds(0, P)], x_s.at[pl.ds(PAD, P)])
        cp_x1 = copy(x_hbm.at[pl.ds(P, S - P)], x_s.at[pl.ds(PAD + P, S - P)])
        cp_wo = [copy(wo_hbm, wo_s.bitcast(BF16))]
        cp_w1 = [copy(w1_hbm, w1_s.bitcast(BF16))]
        cp_w2 = copy(w2_hbm, w2_s.bitcast(BF16))
        cp_w3 = [copy(w3_hbm.at[:, pl.ds(j * LANE, LANE)], w3_s.at[j].bitcast(BF16)) for j in range(F // LANE)]
        cp_w4 = [copy(w4_hbm.at[:, pl.ds(j * LANE, LANE)], w4_s.at[j].bitcast(BF16)) for j in range(NCD)]

        for k in range(NQ):
            cp_w(0, k).start()
        cp_x0.start()
        for cp in cp_mod[:NMA]:
            cp.start()
        for k in range(NQ):
            cp_w(1, k).start()

        cv = jnp.broadcast_to(c_ref[...].astype(F32), (8, D))
        sc = cv * jax.nn.sigmoid(cv)

        def mod(i):
            if i < 2:
                return mod_s[pl.ds(0, 1), pl.ds(i * D, D)]
            n = D // MP
            return jnp.concatenate([modb_s[(i - 2) * n + j, pl.ds(0, 1), :] for j in range(n)], axis=1)

        x_s[pl.ds(0, PAD), :] = jnp.zeros((PAD, D), BF16)
        a_s[...] = jnp.zeros(a_s.shape, F32)
        z_s[...] = jnp.zeros(z_s.shape, U32)
        h_s[pl.ds(0, PAD), :] = jnp.zeros((PAD, D), BF16)
        g_s[pl.ds(0, G0), :] = jnp.zeros((G0, D), F32)
        g_s[pl.ds(G0 + S, 8), :] = jnp.zeros((8, D), F32)

        def relayout(ch, k, us, tie=None):
            for u in us:
                d0 = pl.multiple_of(k * DQ + u * 16, 16)
                v = stage_s[ch % NST][pl.ds(d0, 16), :, :]
                if tie is not None and CFG['tie']:
                    v = v | tie[None]
                v = v.reshape(8, 2, HC // 2, LANE)
                a, b = v[:, 0], v[:, 1]
                lo = (a & 0xFFFF) | (b << 16)
                hi = (a >> 16) | (b & np.uint32(0xFFFF0000))
                t0 = (u % 4) * 144
                for q in range(8):
                    t_s[pl.ds(t0 + q * 9, 8), :] = lo[q]
                    t_s[pl.ds(t0 + 72 + q * 9, 8), :] = hi[q]
                rows = pl.ds(pl.multiple_of(k * (DQ // 2) + u * 8, 8), 8)
                for j in range(HC // 2):
                    wqkv_s[ch][2 * j, rows, :] = t_s[pl.ds(t0 + j, 8, stride=9), :]
                    wqkv_s[ch][2 * j + 1, rows, :] = t_s[pl.ds(t0 + 72 + j, 8, stride=9), :]

        def first_chunk(k, carry):
            cp_w(0, k).wait()
            relayout(0, k, range(DQ // 16))
            return carry
        _loop('first', NQ, first_chunk)
        if NST < NCH:
            for k in range(NQ):
                cp_w(NST, k).start()
        cp_x1.start()

        cp_x0.wait()
        def ln0(i, carry):
            r = pl.multiple_of(i * 128, 128)
            n0_s[pl.ds(r, 128), :] = _ln(x_s[pl.ds(pl.multiple_of(PAD + r, 32), 128), :].astype(F32))
            return carry
        _loop('ln0', P // 128, ln0)
        for j in range(NMA):
            cp_mod[j].wait()
            mod_s[:, pl.ds(MP * j, MP)] = _dot(sc, _bf(wmod_s[j]))
        h0_s[...] = _pk(n0_s[...] * (1.0 + mod(1)) + mod(0))

        for ch in range(NCH):
            last = ch == NCH - 1
            if last:
                cp_x1.wait()
                for cp in cp_mod[NMA:]:
                    cp.wait()

            def bulk(k, carry, ch=ch, last=last):
                if not last:
                    cp_w(ch + 1, k).wait()
                nh = HC // NQ
                nm = (len(cp_mod) - NMA) // NQ
                nr = (S - P) // NQ
                RB = CFG['rb']
                nb = P // RB
                for u in range(nh):
                    j = k * nh + u
                    for t in range(nb):
                        y = _dot(_bf(h0_s[pl.ds(t * RB // 2, RB // 2), :]), _bf(wqkv_s[ch][j]))
                        ring_s[ch * HC + j, pl.ds(OFF + t * RB, RB), :] = y.astype(BF16)
                        piece = u * nb + t
                        tie = pltpu.bitcast(y[:8], U32) & z_s[...]
                        if not last:
                            n = DQ // 16 // (nh * nb)
                            relayout(ch + 1, k, range(piece * n, piece * n + n), tie)
                        else:
                            if piece < nr // 32:
                                r = pl.multiple_of(PAD + P + k * nr + piece * 32, 32)
                                xv = pltpu.bitcast(x_s[pl.ds(r, 32), :], U32) | jnp.tile(tie, (2, NCD))
                                xv = pltpu.bitcast(xv, BF16).astype(F32)
                                h_s[pl.ds(r, 32), :] = (_ln(xv) * (1.0 + mod(1)) + mod(0)).astype(BF16)
                            if piece < nm * MP // LANE:
                                a, b = divmod(piece, MP // LANE)
                                cols = pl.ds(b * LANE, LANE)
                                modb_s[k * nm + a, :, cols] = _dot(sc, _bf(wmod_s[NMA + k * nm + a, :, cols]))
                return carry
            _loop(f'bulk{ch}', NQ, bulk)
            if ch + 1 + NST < NCH:
                for k in range(NQ):
                    cp_w(ch + 1 + NST, k).start()
            if ch == 0:
                for cp in cp_mod[NMA:NMA + 4]:
                    cp.start()
            if ch == 1:
                for cp in cp_mod[NMA + 4:]:
                    cp.start()
            if ch == 2:
                for cp in cp_wo + cp_w1 + [cp_w2]:
                    cp.start()

        for cp in cp_wo + cp_w1 + [cp_w2]:
            cp.wait()
        for cp in cp_w3 + cp_w4:
            cp.start()

        lhs_s[...] = mem0_ref[...].astype(F32)

        row = jax.lax.broadcasted_iota(jnp.int32, (L, L), 0)
        col = jax.lax.broadcasted_iota(jnp.int32, (L, L), 1)

        def seg_rows(base, j):
            r = base + j * SEG
            return r if isinstance(r, int) else pl.multiple_of(r, SEG)

        def post_attention(j):
            r = seg_rows(PAD, j)
            x1 = (x_s[pl.ds(r, SEG), :].astype(F32) + mod(2) * a_s[...]).astype(BF16)
            x_s[pl.ds(r, SEG), :] = x1
            h2 = (_ln(x1.astype(F32)) * (1.0 + mod(4)) + mod(3)).astype(BF16)
            h_s[pl.ds(r, SEG), :] = h2
            return _ln(h2.astype(F32)).astype(BF16)

        def w1_stage(n2, j):
            r = seg_rows(G0, j)
            for n in range(NCD):
                g = _gelu(_dot(n2, _bf(w1_s[:, pl.ds(n * LANE, LANE)])))
                g_s[pl.ds(r, SEG), pl.ds(n * LANE, LANE)] = jnp.where(j >= 0, g, 0.0)

        def w2_stage(j):
            r = seg_rows(G0, j)
            parts = []
            for gi, sh in enumerate((-1, 1, -2, 2)):
                gv = g_s[pl.ds(r - 8, SEG + 16), pl.ds(gi * (D // 4), D // 4)]
                parts.append(gv[8 + sh:8 + sh + SEG].astype(BF16))
            gs = jnp.concatenate(parts, axis=1)
            rp = seg_rows(PAD, j)
            y = h_s[pl.ds(rp, SEG), :].astype(F32) + _dot(gs, _bf(w2_s[...]))
            g_s[pl.ds(seg_rows(G0 - 2 * SEG, j), SEG), :] = x_s[pl.ds(rp, SEG), :].astype(F32) + mod(5) * y
            n = _ln(y)
            hs, hd = SEG // 2, D // 2
            ro = jnp.maximum(j, 0) * (SEG // 4)
            ro = ro if isinstance(j, int) else pl.multiple_of(ro, SEG // 4)
            for i, op in enumerate(_strassen_lhs(n[:hs, :hd], n[:hs, hd:], n[hs:, :hd], n[hs:, hd:])):
                wmod_s[i, pl.ds(ro, SEG // 4), :] = _pk(op)

        def step(s, carry):
            mask = (row >= SEG) | (col >= SEG) | (row >= col)
            wpos = pl.multiple_of(jax.lax.rem(s * R, RING), 8)
            rpos = pl.multiple_of(jax.lax.rem(s * SEG + OFF, RING), SEG)
            tok = h_s[pl.ds(pl.multiple_of(PAD + P + s * R, 8), R), :].astype(F32)
            lhs = jnp.concatenate([tok, lhs_s[...]], axis=0).astype(BF16)
            n2 = post_attention(s - 1)

            def proj(j):
                y = _dot(lhs, _bf(wqkv_s[j // HC][j % HC]))
                ring_s[j, pl.ds(wpos, R), :] = y[:R].astype(BF16)
                return y[R:]

            def full(j, m):
                return jnp.concatenate([ring_s[j, pl.ds(rpos, SEG), :].astype(F32), m], axis=0)

            qs, ks, vs, pr = {}, {}, {}, {}
            for i in range(H + LAG_PV):
                if i < H:
                    qm = proj(i)
                if 0 <= i - LAG_QK < H:
                    hq = i - LAG_QK
                    sco = jnp.where(mask, _dot_nt(qs.pop(hq), ks.pop(hq)) * scale, -1e9)
                    e = jnp.exp(sco - jnp.max(sco, axis=-1, keepdims=True))
                    pr[hq] = e if CFG['post'] else e / jnp.sum(e, axis=-1, keepdims=True)
                if i < H:
                    km = proj(H + i)
                    qs[i] = full(i, qm)
                    ks[i] = full(H + i, km)
                if 0 <= i - LAG_V < H:
                    hv = i - LAG_V
                    vs[hv] = full(2 * H + hv, proj(2 * H + hv))
                if i == CFG['w1']:
                    w1_stage(n2, s - 1)
                if i == H + LAG_V:
                    w2_stage(s - 2)
                if 0 <= i - LAG_PV < H:
                    hp = i - LAG_PV
                    e = pr.pop(hp)
                    o = _dot(e, vs.pop(hp))
                    if CFG['post']:
                        o = o * (1.0 / jnp.sum(e, axis=-1, keepdims=True))
                    o_s[:, pl.ds(hp * LANE, LANE)] = o
            for j in range(NCD):
                y = _dot(o_s[...], _bf(wo_s[:, pl.ds(j * LANE, LANE)]))
                a_s[:, pl.ds(j * LANE, LANE)] = y[:SEG]
                lhs_s[:, pl.ds(j * LANE, LANE)] = y[SEG:]
            return carry

        _loop('steps', NSEG, step)
        w1_stage(post_attention(NSEG - 1), NSEG - 1)
        w2_stage(NSEG - 2)
        w2_stage(NSEG - 1)

        for cp in cp_w3 + cp_w4:
            cp.wait()

        NT = F // 2 // LANE
        HS = S // 2

        def u_op(i, t):
            if i < NCH:
                return wqkv_s[i].at[t]
            return u7_s.at[t]

        def rhs_sums(w, n1, n2, kh):
            b11, b12 = w.at[n1, pl.ds(0, kh)], w.at[n2, pl.ds(0, kh)]
            b21, b22 = w.at[n1, pl.ds(kh, kh)], w.at[n2, pl.ds(kh, kh)]
            for r in range(0, kh, 32):
                rows = pl.ds(r, 32)
                v11, v12, v21, v22 = (_bf(b[rows, :]).astype(F32) for b in (b11, b12, b21, b22))
                for i, v in enumerate((v11 + v22, v12 - v22, v21 - v11, v11 + v12, v21 + v22)):
                    ws_s[i, rows, :] = _pk(v)
            sm = [ws_s.at[i, pl.ds(0, kh)] for i in range(5)]
            return [sm[0], b11, sm[1], sm[2], b22, sm[3], sm[4]]

        def mlp1(t, carry):
            b = rhs_sums(w3_s, t, NT + t, D // 4)
            RB = CFG['rb1']
            for r in range(0, HS, RB):
                rows = pl.ds(r // 2, RB // 2)
                c = _strassen(lambda i: _dot(_bf(wmod_s[i, rows, :]), _bf(b[i][...])))
                for i, op in enumerate(_strassen_lhs(*map(_gelu, c))):
                    u_op(i, t)[rows, :] = _pk(op)
            return carry
        _loop('mlp1', NT, mlp1)

        NH = NCD // 2
        BM = CFG['bm']
        osem = next(sem_i)

        def out_copy(it, half):
            rows = pl.ds(pl.multiple_of((it // NH) * BM, BM), BM)
            cols = pl.ds(pl.multiple_of((it % NH + half * NH) * LANE, LANE), LANE)
            slot = (it % 2) * 2 + half
            return pltpu.make_async_copy(ob_s.at[slot], out_hbm.at[rows, cols], sems.at[osem + slot])

        def mlp2(it, carry):
            @pl.when(it > 1)
            def _():
                out_copy(it - 2, 0).wait()
                out_copy(it - 2, 1).wait()
            blk, n = it // NH, it % NH
            b = rhs_sums(w4_s, n, NH + n, F // 4)
            RB = CFG['rb2']
            for r in range(0, BM // 2, RB):
                rows = pl.ds(pl.multiple_of(blk * (BM // 4) + r // 2, RB // 2), RB // 2)

                def prod(i):
                    lhs = jnp.concatenate([_bf(u_op(i, t)[rows, :]) for t in range(NT)], axis=1)
                    return _dot(lhs, _bf(b[i][...]))
                c11, c12, c21, c22 = _strassen(prod)
                for half, (ct, cb) in enumerate(((c11, c21), (c12, c22))):
                    cols = pl.ds(pl.multiple_of((n + half * NH) * LANE, LANE), LANE)
                    hs = SEG // 2
                    y = jnp.concatenate([v[q:q + hs] for q in range(0, RB, hs) for v in (ct, cb)], axis=0)
                    base = g_s[pl.ds(pl.multiple_of(G0 - 2 * SEG + blk * BM + 2 * r, SEG), 2 * RB), cols]
                    ob_s[(it % 2) * 2 + half, pl.ds(2 * r, 2 * RB), :] = (base + gb_s[n + half * NH, pl.ds(0, 1), :] * y).astype(BF16)
            out_copy(it, 0).start()
            out_copy(it, 1).start()
            return carry
        for n in range(NCD):
            gb_s[n] = jnp.broadcast_to(mod(5)[:, n * LANE:(n + 1) * LANE], (8, LANE))
        nit = (S // BM) * NH
        _loop('mlp2', nit, mlp2)
        for it in (nit - 2, nit - 1):
            out_copy(it, 0).wait()
            out_copy(it, 1).wait()

    scratch = [
        pltpu.VMEM((PAD + S, D), BF16),
        pltpu.VMEM((PAD + S, D), BF16),
        pltpu.VMEM((P // 2, D), U32),
        pltpu.VMEM((H * LANE // 2, D), U32),
        pltpu.VMEM((D // 2, D), U32),
        pltpu.VMEM((D // 2, D), U32),
        pltpu.VMEM((F // LANE, D // 2, LANE), U32),
        pltpu.VMEM((NCD, F // 2, LANE), U32),
        pltpu.VMEM((6 * D // MP, D // 2, MP), U32),
        pltpu.VMEM((3 * H, RING, LANE), BF16),
        pltpu.VMEM((8, 2 * D), F32),
        pltpu.VMEM((4 * D // MP, 8, MP), F32),
        pltpu.VMEM((M, D), F32),
        pltpu.VMEM((L, H * LANE), F32),
        pltpu.VMEM((SEG, D), F32),
        pltpu.VMEM((G0 + S + 8, D), F32),
        pltpu.VMEM((P, D), F32),
        pltpu.VMEM((5, F // 4, LANE), U32),
        pltpu.VMEM((F // 2 // LANE, S // 4, LANE), U32),
        pltpu.VMEM((NCD, 8, LANE), F32),
        pltpu.VMEM((4, CFG['bm'], LANE), BF16),
        pltpu.VMEM((8, LANE), U32),
        pltpu.VMEM((592, LANE), U32),
        pltpu.SemaphoreType.DMA((64,)),
        pltpu.SemaphoreType.DMA((NCH * NQ,)),
    ]
    scratch += [pltpu.VMEM((HC, D // 2, LANE), U32)] * NCH + [pltpu.VMEM((D, HC // 2, LANE), U32)] * NST
    return kernel, scratch


@functools.partial(jax.jit, static_argnames=("A_seg_len",))
def pallas_adaLN_cond__memory_aug_recurrent_mem_tr__mixer_s_mlp__prompt_kernel(
    A_x: jax.Array,
    A_mem0: jax.Array,
    A_Wq: jax.Array,
    A_Wk: jax.Array,
    A_Wv: jax.Array,
    A_Wo: jax.Array,
    A_seg_len: int,
    B_x: jax.Array,
    B_w1: jax.Array,
    B_w2: jax.Array,
    B_w3: jax.Array,
    B_w4: jax.Array,
    c: jax.Array,
    w_mod: jax.Array,
):
    del B_x
    B, S, D = A_x.shape
    _, H, Dh = A_Wq.shape
    M = A_mem0.shape[1]
    F = B_w3.shape[1]
    assert B == 1 and Dh == LANE
    kernel, scratch = _make_kernel(S, D, H, M, int(A_seg_len), F)
    hbm = pl.BlockSpec(memory_space=pl.ANY)
    vmem = pl.BlockSpec(memory_space=pltpu.VMEM)
    out = pl.pallas_call(
        kernel,
        in_specs=[hbm, vmem, hbm, hbm, hbm, hbm, hbm, hbm, hbm, hbm, vmem, hbm],
        out_specs=hbm,
        out_shape=jax.ShapeDtypeStruct((S, D), A_x.dtype),
        scratch_shapes=scratch,
        compiler_params=pltpu.CompilerParams(vmem_limit_bytes=127 * 1024 * 1024, flags={0: None, 1: {'XLA_TPU_FORCE_LP_LLO_SCHEDULER': True}, 2: {'XLA_TPU_EVENLY_DISTRIBUTE_CRITICAL_NODES': True}}[CFG['fl']]),
    )(A_x.reshape(S, D), A_mem0.reshape(M, D), A_Wq, A_Wk, A_Wv, A_Wo.reshape(H * Dh, D),
      B_w1, B_w2, B_w3, B_w4, c, w_mod)
    return out.reshape(B, S, D)
```

```python
import contextlib
import functools

import jax
import jax.numpy as jnp
import numpy as np
import jax.experimental.pallas as pl
import jax.experimental.pallas.tpu as pltpu

F32 = jnp.float32
BF16 = jnp.bfloat16
U32 = jnp.uint32
LANE = 128
CFG = dict(qk=2, v=3, pv=5, post=0, rb=128, fl=2, tie=1, prof=0, nsub=1, nt=20, w1=8, rb1=128, rb2=512, bm=1024)


def _scope(n):
    return jax.named_scope(n) if CFG['prof'] else contextlib.nullcontext()


def _loop(name, n, body):
    with _scope(name):
        jax.lax.fori_loop(0, n, body, 0)


def _dot(a, b):
    return jax.lax.dot_general(a, b, (((1,), (0,)), ((), ())), preferred_element_type=F32)


def _dot_nt(a, b):
    return jax.lax.dot_general(a, b, (((1,), (1,)), ((), ())), preferred_element_type=F32)


def _bf(w):
    return pltpu.bitcast(w, BF16)


def _pk(x):
    return pltpu.bitcast(x.astype(BF16), U32)


def _ln(x):
    m = jnp.mean(x, axis=-1, keepdims=True)
    xc = x - m
    v = jnp.mean(xc * xc, axis=-1, keepdims=True)
    return xc * jax.lax.rsqrt(v + 1e-5)


def _gelu(x):
    return jax.nn.gelu(x, approximate=True)


def _strassen_lhs(a11, a12, a21, a22):
    return a11 + a22, a21 + a22, a11, a22, a11 + a12, a21 - a11, a12 - a22


def _strassen(prod):
    m2 = prod(1)
    m5 = prod(4)
    m4 = prod(3)
    c21 = m2 + m4
    c11 = m4 - m5
    m3 = prod(2)
    c12 = m3 + m5
    c22 = m3 - m2
    m1 = prod(0)
    c11 = c11 + m1
    c22 = c22 + m1
    c11 = c11 + prod(6)
    c22 = c22 + prod(5)
    return c11, c12, c21, c22


def _make_kernel(S, D, H, M, SEG, F):
    NSEG = S // SEG
    R = SEG - M
    P = S - R * NSEG
    RING = 576
    OFF = RING - P
    L = SEG + M
    NCD = D // LANE
    PAD = 2 * SEG
    G0 = 4 * SEG
    LAG_QK, LAG_V, LAG_PV = CFG['qk'], CFG['v'], CFG['pv']
    scale = float(LANE) ** -0.5

    DK = 2 * LANE
    NKB = D // DK
    NPC = 3 * NKB
    NSUB = CFG['nsub']
    NST = 4
    MP = 2 * DK

    def kernel(x_hbm, mem0_ref, wq_hbm, wk_hbm, wv_hbm, wo_hbm, w1_hbm, w2_hbm, w3_hbm, w4_hbm, c_ref, wmod_hbm,
               out_hbm,
               x_s, h_s, h0_s, wqkv_s, wo_s, w1_s, w2_s, w3_s, w4_s, wmod_s, stage_s, ring_s, mod_s, tok_s, lhs_s,
               o_s, a_s, g_s, n0_s, ws_s, u7_s, gb_s, ob_s, z_s, t_s, sems, wsems, msems):
        sem_i = iter(range(64))

        def copy(src, dst):
            return pltpu.make_async_copy(src, dst, sems.at[next(sem_i)])

        def cp_w(pc, q, w=wq_hbm):
            n = DK // NSUB
            src = w.at[pl.ds((pc % NKB) * DK + q * n, n)]
            dst = stage_s.at[pc % NST, pl.ds(q * n, n)].bitcast(BF16)
            return pltpu.make_async_copy(src, dst, wsems.at[(pc % NST) * NSUB + q])

        def cp_mod(j, q):
            col = jnp.where(j < NKB, q * D + j * DK, j * MP + q * DK)
            src = wmod_hbm.at[:, pl.ds(pl.multiple_of(col, DK), DK)]
            return pltpu.make_async_copy(src, wmod_s.at[j, :, pl.ds(q * DK, DK)].bitcast(BF16), msems.at[2 * j + q])

        def start_piece(pc):
            for t, w in enumerate((wq_hbm, wk_hbm, wv_hbm)):
                @pl.when(pc // NKB == t)
                def _():
                    for q in range(NSUB):
                        cp_w(pc, q, w).start()

        def start_mod(j):
            cp_mod(j, 0).start()
            cp_mod(j, 1).start()

        cp_x0 = copy(x_hbm.at[pl.ds(0, P)], x_s.at[pl.ds(PAD, P)])
        CH = 512
        late = [copy(x_hbm.at[pl.ds(r, CH)], x_s.at[pl.ds(PAD + r, CH)]) for r in range(P, S, CH)]
        for src, dst in ((w1_hbm, w1_s), (w2_hbm, w2_s), (wo_hbm, wo_s)):
            late += [copy(src.at[pl.ds(r, CH)], dst.at[pl.ds(r // 2, CH // 2)].bitcast(BF16))
                     for r in range(0, src.shape[0], CH)]
        cp_w3 = [copy(w3_hbm.at[:, pl.ds(j * LANE, LANE)], w3_s.at[j].bitcast(BF16)) for j in range(F // LANE)]
        cp_w4 = [copy(w4_hbm.at[:, pl.ds(j * LANE, LANE)], w4_s.at[j].bitcast(BF16)) for j in range(NCD)]

        cp_x0.start()
        for q in range(NSUB):
            cp_w(0, q).start()
        start_mod(0)

        cv = jnp.broadcast_to(c_ref[...].astype(F32), (8, D))
        sc = cv * jax.nn.sigmoid(cv)

        def mod(i):
            if i < 2:
                return jnp.concatenate([mod_s[j, pl.ds(0, 1), pl.ds(i * DK, DK)] for j in range(NKB)], axis=1)
            n = D // MP
            return jnp.concatenate([mod_s[i * n + j, pl.ds(0, 1), :] for j in range(n)], axis=1)

        x_s[pl.ds(0, PAD), :] = jnp.zeros((PAD, D), BF16)
        h_s[pl.ds(0, PAD), :] = jnp.zeros((PAD, D), BF16)
        a_s[...] = jnp.zeros(a_s.shape, F32)
        z_s[...] = jnp.zeros(z_s.shape, U32)
        g_s[pl.ds(0, G0), :] = jnp.zeros((G0, D), F32)
        g_s[pl.ds(G0 + S, 8), :] = jnp.zeros((8, D), F32)

        def relayout(pc, u, tie=None):
            d0, hg = (u // 2) * 16, u % 2
            v = stage_s[pc % NST, pl.ds(d0, 16), pl.ds(hg * 8, 8), :]
            if tie is not None:
                v = v | tie[None]
            v = v.reshape(8, 2, 8, LANE)
            a, b = v[:, 0], v[:, 1]
            lo = (a & 0xFFFF) | (b << 16)
            hi = (a >> 16) | (b & np.uint32(0xFFFF0000))
            t0 = (u % 4) * 144
            for q in range(8):
                t_s[pl.ds(t0 + q * 9, 8), :] = lo[q]
                t_s[pl.ds(t0 + 72 + q * 9, 8), :] = hi[q]
            rows = pl.ds(pl.multiple_of((pc % NKB) * (DK // 2) + d0 // 2, 8), 8)
            head = (pc // NKB) * H + hg * 16
            for j in range(8):
                wqkv_s[head + 2 * j, rows, :] = t_s[pl.ds(t0 + j, 8, stride=9), :]
                wqkv_s[head + 2 * j + 1, rows, :] = t_s[pl.ds(t0 + 72 + j, 8, stride=9), :]

        NU = DK // 16 * 2

        def mod_cols(j, b):
            cols = pl.ds(b * LANE, LANE)
            mod_s[j, :, cols] = _dot(sc, _bf(wmod_s[j, :, cols]))

        def modulate(j):
            cp_mod(j, 0).wait()
            cp_mod(j, 1).wait()
            for b in range(MP // LANE):
                mod_cols(j, b)
            m = mod_s[j, pl.ds(0, 1), :]
            for r in range(0, P, 64):
                hv = n0_s[j, pl.ds(r, 64), :] * (1.0 + m[:, DK:]) + m[:, :DK]
                h0_s[j, pl.ds(r // 2, 32), :] = _pk(hv)

        cp_x0.wait()
        for q in range(NSUB):
            cp_w(1, q).start()

        def ln0(i, carry):
            r = pl.multiple_of(i * 128, 128)
            n = _ln(x_s[pl.ds(pl.multiple_of(PAD + r, 32), 128), :].astype(F32))
            for j in range(NKB):
                n0_s[j, pl.ds(r, 128), :] = n[:, j * DK:(j + 1) * DK]
            return carry
        _loop('ln0', P // 128, ln0)
        with _scope('first'):
            for u in range(NU):
                if u % (NU // NSUB) == 0:
                    cp_w(0, u // (NU // NSUB)).wait()
                relayout(0, u)

        def bulk(pc, carry):
            pl.when(pc < NKB)(lambda: modulate(pc))
            more = pc + 1 < NPC
            nxt = jnp.minimum(pc + 1, NPC - 1)
            for q in range(NSUB):
                pl.when(more)(cp_w(nxt, q).wait)
            for q in range(2):
                pl.when(pc >= NKB)(cp_mod(pc, q).wait)
            pl.when(more)(lambda: start_mod(pc + 1))
            pl.when(pc + 2 < NPC)(lambda: start_piece(pc + 2))
            for i, cp in enumerate(late):
                pl.when(pc == (i if i < NPC - 2 else NPC - 2 + (i - NPC + 2) // 3))(cp.start)

            kb = pc % NKB
            rows = pl.ds(pl.multiple_of(kb * (DK // 2), DK // 2), DK // 2)
            RB = CFG['rb']
            for hd in range(H):
                j = (pc // NKB) * H + hd
                for r in range(0, P, RB):
                    acc = g_s.at[pl.ds(G0 + (hd // NCD) * P + r, RB), pl.ds((hd % NCD) * LANE, LANE)]
                    y = _dot(_bf(h0_s[kb, pl.ds(r // 2, RB // 2), :]), _bf(wqkv_s[j, rows, :]))
                    if r == 0:
                        tie = pltpu.bitcast(y[:8], U32) & z_s[...]
                    y = y + jnp.where(kb > 0, acc[...], 0.0)
                    acc[...] = y
                    ring_s[j, pl.ds(OFF + r, RB), :] = y.astype(BF16)
                relayout(nxt, hd, tie)
                if hd % 8 == 4:
                    mod_cols(pc, hd // 8)
            return carry
        _loop('bulk', NPC, bulk)

        with _scope('late'):
            for cp in late:
                cp.wait()
        for cp in cp_w3 + cp_w4:
            cp.start()

        def next_tokens(s):
            r = PAD + P + s * R
            xv = x_s[pl.ds(r if isinstance(r, int) else pl.multiple_of(r, 8), R), :].astype(F32)
            tok_s[...] = _ln(xv) * (1.0 + mod(1)) + mod(0)

        next_tokens(0)
        lhs_s[...] = mem0_ref[...].astype(F32)

        row = jax.lax.broadcasted_iota(jnp.int32, (L, L), 0)
        col = jax.lax.broadcasted_iota(jnp.int32, (L, L), 1)

        def seg_rows(base, j):
            r = base + j * SEG
            return r if isinstance(r, int) else pl.multiple_of(r, SEG)

        def post_attention(j):
            r = seg_rows(PAD, j)
            x1 = (x_s[pl.ds(r, SEG), :].astype(F32) + mod(2) * a_s[...]).astype(BF16)
            x_s[pl.ds(r, SEG), :] = x1
            h2 = (_ln(x1.astype(F32)) * (1.0 + mod(4)) + mod(3)).astype(BF16)
            h_s[pl.ds(r, SEG), :] = h2
            return _ln(h2.astype(F32)).astype(BF16)

        def w1_stage(n2, j):
            r = seg_rows(G0, j)
            for n in range(NCD):
                g = _gelu(_dot(n2, _bf(w1_s[:, pl.ds(n * LANE, LANE)])))
                g_s[pl.ds(r, SEG), pl.ds(n * LANE, LANE)] = jnp.where(j >= 0, g, 0.0)

        def w2_stage(j):
            r = seg_rows(G0, j)
            parts = []
            for gi, sh in enumerate((-1, 1, -2, 2)):
                gv = g_s[pl.ds(r - 8, SEG + 16), pl.ds(gi * (D // 4), D // 4)]
                parts.append(gv[8 + sh:8 + sh + SEG].astype(BF16))
            gs = jnp.concatenate(parts, axis=1)
            rp = seg_rows(PAD, j)
            y = h_s[pl.ds(rp, SEG), :].astype(F32) + _dot(gs, _bf(w2_s[...]))
            g_s[pl.ds(seg_rows(G0 - 2 * SEG, j), SEG), :] = x_s[pl.ds(rp, SEG), :].astype(F32) + mod(5) * y
            n = _ln(y)
            hs, hd = SEG // 2, D // 2
            ro = jnp.maximum(j, 0) * (SEG // 4)
            ro = ro if isinstance(j, int) else pl.multiple_of(ro, SEG // 4)
            for i, op in enumerate(_strassen_lhs(n[:hs, :hd], n[:hs, hd:], n[hs:, :hd], n[hs:, hd:])):
                wmod_s[i, pl.ds(ro, SEG // 4), :] = _pk(op)

        def step(s, carry):
            mask = (row >= SEG) | (col >= SEG) | (row >= col)
            wpos = pl.multiple_of(jax.lax.rem(s * R, RING), 8)
            rpos = pl.multiple_of(jax.lax.rem(s * SEG + OFF, RING), SEG)
            lhs = jnp.concatenate([tok_s[...], lhs_s[...]], axis=0).astype(BF16)
            n2 = post_attention(s - 1)

            def proj(j):
                y = _dot(lhs, _bf(wqkv_s[j]))
                ring_s[j, pl.ds(wpos, R), :] = y[:R].astype(BF16)
                return y[R:]

            def full(j, m):
                return jnp.concatenate([ring_s[j, pl.ds(rpos, SEG), :].astype(F32), m], axis=0)

            qs, ks, vs, pr = {}, {}, {}, {}
            for i in range(H + LAG_PV):
                if i < H:
                    qm = proj(i)
                if 0 <= i - LAG_QK < H:
                    hq = i - LAG_QK
                    sco = jnp.where(mask, _dot_nt(qs.pop(hq), ks.pop(hq)) * scale, -1e9)
                    e = jnp.exp(sco - jnp.max(sco, axis=-1, keepdims=True))
                    pr[hq] = e if CFG['post'] else e / jnp.sum(e, axis=-1, keepdims=True)
                if i < H:
                    km = proj(H + i)
                    qs[i] = full(i, qm)
                    ks[i] = full(H + i, km)
                if 0 <= i - LAG_V < H:
                    hv = i - LAG_V
                    vs[hv] = full(2 * H + hv, proj(2 * H + hv))
                if i == CFG['nt']:
                    next_tokens(jnp.minimum(s + 1, NSEG - 1))
                if i == CFG['w1']:
                    w1_stage(n2, s - 1)
                if i == H + LAG_V:
                    w2_stage(s - 2)
                if 0 <= i - LAG_PV < H:
                    hp = i - LAG_PV
                    e = pr.pop(hp)
                    o = _dot(e, vs.pop(hp))
                    if CFG['post']:
                        o = o * (1.0 / jnp.sum(e, axis=-1, keepdims=True))
                    o_s[:, pl.ds(hp * LANE, LANE)] = o
            for j in range(NCD):
                y = _dot(o_s[...], _bf(wo_s[:, pl.ds(j * LANE, LANE)]))
                a_s[:, pl.ds(j * LANE, LANE)] = y[:SEG]
                lhs_s[:, pl.ds(j * LANE, LANE)] = y[SEG:]
            return carry

        _loop('steps', NSEG, step)
        w1_stage(post_attention(NSEG - 1), NSEG - 1)
        w2_stage(NSEG - 2)
        w2_stage(NSEG - 1)

        for cp in cp_w3 + cp_w4:
            cp.wait()

        NT = F // 2 // LANE
        HS = S // 2

        def u_op(i, t):
            if i < 6:
                return wqkv_s.at[i * 16 + t]
            return u7_s.at[t]

        def rhs_sums(w, n1, n2, kh):
            b11, b12 = w.at[n1, pl.ds(0, kh)], w.at[n2, pl.ds(0, kh)]
            b21, b22 = w.at[n1, pl.ds(kh, kh)], w.at[n2, pl.ds(kh, kh)]
            for r in range(0, kh, 32):
                rows = pl.ds(r, 32)
                v11, v12, v21, v22 = (_bf(b[rows, :]).astype(F32) for b in (b11, b12, b21, b22))
                for i, v in enumerate((v11 + v22, v12 - v22, v21 - v11, v11 + v12, v21 + v22)):
                    ws_s[i, rows, :] = _pk(v)
            sm = [ws_s.at[i, pl.ds(0, kh)] for i in range(5)]
            return [sm[0], b11, sm[1], sm[2], b22, sm[3], sm[4]]

        def mlp1(t, carry):
            b = rhs_sums(w3_s, t, NT + t, D // 4)
            RB = CFG['rb1']
            for r in range(0, HS, RB):
                rows = pl.ds(r // 2, RB // 2)
                c = _strassen(lambda i: _dot(_bf(wmod_s[i, rows, :]), _bf(b[i][...])))
                for i, op in enumerate(_strassen_lhs(*map(_gelu, c))):
                    u_op(i, t)[rows, :] = _pk(op)
            return carry
        _loop('mlp1', NT, mlp1)

        NH = NCD // 2
        BM = CFG['bm']
        osem = next(sem_i)

        def out_copy(it, half):
            rows = pl.ds(pl.multiple_of((it // NH) * BM, BM), BM)
            cols = pl.ds(pl.multiple_of((it % NH + half * NH) * LANE, LANE), LANE)
            slot = (it % 2) * 2 + half
            return pltpu.make_async_copy(ob_s.at[slot], out_hbm.at[rows, cols], sems.at[osem + slot])

        def mlp2(it, carry):
            @pl.when(it > 1)
            def _():
                out_copy(it - 2, 0).wait()
                out_copy(it - 2, 1).wait()
            blk, n = it // NH, it % NH
            b = rhs_sums(w4_s, n, NH + n, F // 4)
            RB = CFG['rb2']
            for r in range(0, BM // 2, RB):
                rows = pl.ds(pl.multiple_of(blk * (BM // 4) + r // 2, RB // 2), RB // 2)

                def prod(i):
                    lhs = jnp.concatenate([_bf(u_op(i, t)[rows, :]) for t in range(NT)], axis=1)
                    return _dot(lhs, _bf(b[i][...]))
                c11, c12, c21, c22 = _strassen(prod)
                for half, (ct, cb) in enumerate(((c11, c21), (c12, c22))):
                    cols = pl.ds(pl.multiple_of((n + half * NH) * LANE, LANE), LANE)
                    hs = SEG // 2
                    y = jnp.concatenate([v[q:q + hs] for q in range(0, RB, hs) for v in (ct, cb)], axis=0)
                    base = g_s[pl.ds(pl.multiple_of(G0 - 2 * SEG + blk * BM + 2 * r, SEG), 2 * RB), cols]
                    ob_s[(it % 2) * 2 + half, pl.ds(2 * r, 2 * RB), :] = (base + gb_s[n + half * NH, pl.ds(0, 1), :] * y).astype(BF16)
            out_copy(it, 0).start()
            out_copy(it, 1).start()
            return carry
        for n in range(NCD):
            gb_s[n] = jnp.broadcast_to(mod(5)[:, n * LANE:(n + 1) * LANE], (8, LANE))
        nit = (S // BM) * NH
        _loop('mlp2', nit, mlp2)
        for it in (nit - 2, nit - 1):
            out_copy(it, 0).wait()
            out_copy(it, 1).wait()

    scratch = [
        pltpu.VMEM((PAD + S, D), BF16),
        pltpu.VMEM((PAD + S, D), BF16),
        pltpu.VMEM((NKB, P // 2, DK), U32),
        pltpu.VMEM((3 * H, D // 2, LANE), U32),
        pltpu.VMEM((H * LANE // 2, D), U32),
        pltpu.VMEM((D // 2, D), U32),
        pltpu.VMEM((D // 2, D), U32),
        pltpu.VMEM((F // LANE, D // 2, LANE), U32),
        pltpu.VMEM((NCD, F // 2, LANE), U32),
        pltpu.VMEM((6 * D // MP, D // 2, MP), U32),
        pltpu.VMEM((NST, DK, H // 2, LANE), U32),
        pltpu.VMEM((3 * H, RING, LANE), BF16),
        pltpu.VMEM((6 * D // MP, 8, MP), F32),
        pltpu.VMEM((R, D), F32),
        pltpu.VMEM((M, D), F32),
        pltpu.VMEM((L, H * LANE), F32),
        pltpu.VMEM((SEG, D), F32),
        pltpu.VMEM((G0 + S + 8, D), F32),
        pltpu.VMEM((NKB, P, DK), F32),
        pltpu.VMEM((5, F // 4, LANE), U32),
        pltpu.VMEM((F // 2 // LANE, S // 4, LANE), U32),
        pltpu.VMEM((NCD, 8, LANE), F32),
        pltpu.VMEM((4, CFG['bm'], LANE), BF16),
        pltpu.VMEM((8, LANE), U32),
        pltpu.VMEM((592, LANE), U32),
        pltpu.SemaphoreType.DMA((64,)),
        pltpu.SemaphoreType.DMA((NST * NSUB,)),
        pltpu.SemaphoreType.DMA((12 * D // MP,)),
    ]
    return kernel, scratch


@functools.partial(jax.jit, static_argnames=("A_seg_len",))
def pallas_adaLN_cond__memory_aug_recurrent_mem_tr__mixer_s_mlp__prompt_kernel(
    A_x: jax.Array,
    A_mem0: jax.Array,
    A_Wq: jax.Array,
    A_Wk: jax.Array,
    A_Wv: jax.Array,
    A_Wo: jax.Array,
    A_seg_len: int,
    B_x: jax.Array,
    B_w1: jax.Array,
    B_w2: jax.Array,
    B_w3: jax.Array,
    B_w4: jax.Array,
    c: jax.Array,
    w_mod: jax.Array,
):
    del B_x
    B, S, D = A_x.shape
    _, H, Dh = A_Wq.shape
    M = A_mem0.shape[1]
    F = B_w3.shape[1]
    assert B == 1 and Dh == LANE
    kernel, scratch = _make_kernel(S, D, H, M, int(A_seg_len), F)
    hbm = pl.BlockSpec(memory_space=pl.ANY)
    vmem = pl.BlockSpec(memory_space=pltpu.VMEM)
    out = pl.pallas_call(
        kernel,
        in_specs=[hbm, vmem, hbm, hbm, hbm, hbm, hbm, hbm, hbm, hbm, vmem, hbm],
        out_specs=hbm,
        out_shape=jax.ShapeDtypeStruct((S, D), A_x.dtype),
        scratch_shapes=scratch,
        compiler_params=pltpu.CompilerParams(vmem_limit_bytes=127 * 1024 * 1024, flags={0: None, 1: {'XLA_TPU_FORCE_LP_LLO_SCHEDULER': True}, 2: {'XLA_TPU_EVENLY_DISTRIBUTE_CRITICAL_NODES': True}}[CFG['fl']]),
    )(A_x.reshape(S, D), A_mem0.reshape(M, D), A_Wq, A_Wk, A_Wv, A_Wo.reshape(H * Dh, D),
      B_w1, B_w2, B_w3, B_w4, c, w_mod)
    return out.reshape(B, S, D)
```

```python
import contextlib
import functools

import jax
import jax.numpy as jnp
import numpy as np
import jax.experimental.pallas as pl
import jax.experimental.pallas.tpu as pltpu

F32 = jnp.float32
BF16 = jnp.bfloat16
U32 = jnp.uint32
LANE = 128
CFG = dict(qk=2, v=3, pv=5, post=0, rb=128, fl=2, tie=1, prof=0, us=2, um=2, nsub=1, j0=0, j1=7, j2=14, j3=22, jl=6, j4=3, w1=8, rb1=128, rb2=512, bm=1024)


def _scope(n):
    return jax.named_scope(n) if CFG['prof'] else contextlib.nullcontext()


def _loop(name, n, body, unroll=1):
    def group(i, carry):
        for u in range(unroll):
            body(i * unroll + u, carry)
        return carry
    with _scope(name):
        jax.lax.fori_loop(0, n // unroll, group, 0)


def _dot(a, b):
    return jax.lax.dot_general(a, b, (((1,), (0,)), ((), ())), preferred_element_type=F32)


def _dot_nt(a, b):
    return jax.lax.dot_general(a, b, (((1,), (1,)), ((), ())), preferred_element_type=F32)


def _bf(w):
    return pltpu.bitcast(w, BF16)


def _pk(x):
    return pltpu.bitcast(x.astype(BF16), U32)


def _ln(x):
    m = jnp.mean(x, axis=-1, keepdims=True)
    xc = x - m
    v = jnp.mean(xc * xc, axis=-1, keepdims=True)
    return xc * jax.lax.rsqrt(v + 1e-5)


def _gelu(x):
    return jax.nn.gelu(x, approximate=True)


def _strassen_lhs(a11, a12, a21, a22):
    return a11 + a22, a21 + a22, a11, a22, a11 + a12, a21 - a11, a12 - a22


def _strassen(prod):
    m2 = prod(1)
    m5 = prod(4)
    m4 = prod(3)
    c21 = m2 + m4
    c11 = m4 - m5
    m3 = prod(2)
    c12 = m3 + m5
    c22 = m3 - m2
    m1 = prod(0)
    c11 = c11 + m1
    c22 = c22 + m1
    c11 = c11 + prod(6)
    c22 = c22 + prod(5)
    return c11, c12, c21, c22


def _make_kernel(S, D, H, M, SEG, F):
    NSEG = S // SEG
    R = SEG - M
    P = S - R * NSEG
    RING = 576
    OFF = RING - P
    L = SEG + M
    NCD = D // LANE
    PAD = 3 * SEG
    G0 = 5 * SEG
    LAG_QK, LAG_V, LAG_PV = CFG['qk'], CFG['v'], CFG['pv']
    scale = float(LANE) ** -0.5

    DK = 2 * LANE
    NKB = D // DK
    NPC = 3 * NKB
    NSUB = CFG['nsub']
    NST = 4
    MP = 2 * DK

    def kernel(x_hbm, mem0_ref, wq_hbm, wk_hbm, wv_hbm, wo_hbm, w1_hbm, w2_hbm, w3_hbm, w4_hbm, c_ref, wmod_hbm,
               out_hbm,
               x_s, h_s, h0_s, wqkv_s, wo_s, w1_s, w2_s, w3_s, w4_s, wmod_s, stage_s, ring_s, mod_s, tok_s, lhs_s,
               o_s, a_s, n2_s, g_s, n0_s, ws_s, u7_s, gb_s, ob_s, z_s, t_s, sems, wsems, msems):
        sem_i = iter(range(64))

        def copy(src, dst):
            return pltpu.make_async_copy(src, dst, sems.at[next(sem_i)])

        def cp_w(pc, q, w=wq_hbm):
            n = DK // NSUB
            src = w.at[pl.ds((pc % NKB) * DK + q * n, n)]
            dst = stage_s.at[pc % NST, pl.ds(q * n, n)].bitcast(BF16)
            return pltpu.make_async_copy(src, dst, wsems.at[(pc % NST) * NSUB + q])

        def cp_mod(j, q):
            col = jnp.where(j < NKB, q * D + j * DK, j * MP + q * DK)
            src = wmod_hbm.at[:, pl.ds(pl.multiple_of(col, DK), DK)]
            return pltpu.make_async_copy(src, wmod_s.at[j, :, pl.ds(q * DK, DK)].bitcast(BF16), msems.at[2 * j + q])

        def start_piece(pc):
            for t, w in enumerate((wq_hbm, wk_hbm, wv_hbm)):
                @pl.when(pc // NKB == t)
                def _():
                    for q in range(NSUB):
                        cp_w(pc, q, w).start()

        def start_mod(j):
            cp_mod(j, 0).start()
            cp_mod(j, 1).start()

        cp_x0 = copy(x_hbm.at[pl.ds(0, P)], x_s.at[pl.ds(PAD, P)])
        CH = 512
        late = [copy(x_hbm.at[pl.ds(r, CH)], x_s.at[pl.ds(PAD + r, CH)]) for r in range(P, S, CH)]
        for src, dst in ((w1_hbm, w1_s), (w2_hbm, w2_s), (wo_hbm, wo_s)):
            late += [copy(src.at[pl.ds(r, CH)], dst.at[pl.ds(r // 2, CH // 2)].bitcast(BF16))
                     for r in range(0, src.shape[0], CH)]
        cp_w3 = [copy(w3_hbm.at[:, pl.ds(j * LANE, LANE)], w3_s.at[j].bitcast(BF16)) for j in range(F // LANE)]
        cp_w4 = [copy(w4_hbm.at[:, pl.ds(j * LANE, LANE)], w4_s.at[j].bitcast(BF16)) for j in range(NCD)]

        cp_x0.start()
        for q in range(NSUB):
            cp_w(0, q).start()
        start_mod(0)

        cv = jnp.broadcast_to(c_ref[...].astype(F32), (8, D))
        sc = cv * jax.nn.sigmoid(cv)

        def mod(i):
            if i < 2:
                return jnp.concatenate([mod_s[j, pl.ds(0, 1), pl.ds(i * DK, DK)] for j in range(NKB)], axis=1)
            n = D // MP
            return jnp.concatenate([mod_s[i * n + j, pl.ds(0, 1), :] for j in range(n)], axis=1)

        x_s[pl.ds(0, PAD), :] = jnp.zeros((PAD, D), BF16)
        h_s[pl.ds(0, PAD), :] = jnp.zeros((PAD, D), BF16)
        a_s[...] = jnp.zeros(a_s.shape, F32)
        z_s[...] = jnp.zeros(z_s.shape, U32)
        g_s[pl.ds(0, G0), :] = jnp.zeros((G0, D), F32)
        g_s[pl.ds(G0 + S, 8), :] = jnp.zeros((8, D), F32)

        def relayout(pc, u, tie=None):
            d0, hg = (u // 2) * 16, u % 2
            v = stage_s[pc % NST, pl.ds(d0, 16), pl.ds(hg * 8, 8), :]
            if tie is not None:
                v = v | tie[None]
            v = v.reshape(8, 2, 8, LANE)
            a, b = v[:, 0], v[:, 1]
            lo = (a & 0xFFFF) | (b << 16)
            hi = (a >> 16) | (b & np.uint32(0xFFFF0000))
            t0 = (u % 4) * 144
            for q in range(8):
                t_s[pl.ds(t0 + q * 9, 8), :] = lo[q]
                t_s[pl.ds(t0 + 72 + q * 9, 8), :] = hi[q]
            rows = pl.ds(pl.multiple_of((pc % NKB) * (DK // 2) + d0 // 2, 8), 8)
            head = (pc // NKB) * H + hg * 16
            for j in range(8):
                wqkv_s[head + 2 * j, rows, :] = t_s[pl.ds(t0 + j, 8, stride=9), :]
                wqkv_s[head + 2 * j + 1, rows, :] = t_s[pl.ds(t0 + 72 + j, 8, stride=9), :]

        NU = DK // 16 * 2

        def mod_cols(j, b):
            cols = pl.ds(b * LANE, LANE)
            mod_s[j, :, cols] = _dot(sc, _bf(wmod_s[j, :, cols]))

        def modulate(j):
            cp_mod(j, 0).wait()
            cp_mod(j, 1).wait()
            for b in range(MP // LANE):
                mod_cols(j, b)
            m = mod_s[j, pl.ds(0, 1), :]
            for r in range(0, P, 64):
                hv = n0_s[j, pl.ds(r, 64), :] * (1.0 + m[:, DK:]) + m[:, :DK]
                h0_s[j, pl.ds(r // 2, 32), :] = _pk(hv)

        cp_x0.wait()
        for q in range(NSUB):
            cp_w(1, q).start()

        def ln0(i, carry):
            r = pl.multiple_of(i * 128, 128)
            n = _ln(x_s[pl.ds(pl.multiple_of(PAD + r, 32), 128), :].astype(F32))
            for j in range(NKB):
                n0_s[j, pl.ds(r, 128), :] = n[:, j * DK:(j + 1) * DK]
            return carry
        _loop('ln0', P // 128, ln0)
        with _scope('first'):
            for u in range(NU):
                if u % (NU // NSUB) == 0:
                    cp_w(0, u // (NU // NSUB)).wait()
                relayout(0, u)

        def bulk(pc, carry):
            pl.when(pc < NKB)(lambda: modulate(pc))
            more = pc + 1 < NPC
            nxt = jnp.minimum(pc + 1, NPC - 1)
            for q in range(NSUB):
                pl.when(more)(cp_w(nxt, q).wait)
            for q in range(2):
                pl.when(pc >= NKB)(cp_mod(pc, q).wait)
            pl.when(more)(lambda: start_mod(pc + 1))
            pl.when(pc + 2 < NPC)(lambda: start_piece(pc + 2))
            for i, cp in enumerate(late):
                pl.when(pc == (i if i < NPC - 2 else NPC - 2 + (i - NPC + 2) // 3))(cp.start)

            kb = pc % NKB
            rows = pl.ds(pl.multiple_of(kb * (DK // 2), DK // 2), DK // 2)
            RB = CFG['rb']
            for hd in range(H):
                j = (pc // NKB) * H + hd
                for r in range(0, P, RB):
                    acc = g_s.at[pl.ds(G0 + (hd // NCD) * P + r, RB), pl.ds((hd % NCD) * LANE, LANE)]
                    y = _dot(_bf(h0_s[kb, pl.ds(r // 2, RB // 2), :]), _bf(wqkv_s[j, rows, :]))
                    if r == 0:
                        tie = pltpu.bitcast(y[:8], U32) & z_s[...]
                    y = y + jnp.where(kb > 0, acc[...], 0.0)
                    acc[...] = y
                    ring_s[j, pl.ds(OFF + r, RB), :] = y.astype(BF16)
                relayout(nxt, hd, tie)
                if hd % 8 == 4:
                    mod_cols(pc, hd // 8)
            return carry
        _loop('bulk', NPC, bulk)

        with _scope('late'):
            for cp in late:
                cp.wait()
        for cp in cp_w3 + cp_w4:
            cp.start()

        def next_tokens(s):
            r = PAD + P + s * R
            xv = x_s[pl.ds(r if isinstance(r, int) else pl.multiple_of(r, 8), R), :].astype(F32)
            t = _ln(xv) * (1.0 + mod(1)) + mod(0)
            tok_s[...] = t
            return t

        next_tokens(0)
        lhs_s[...] = mem0_ref[...].astype(F32)

        row = jax.lax.broadcasted_iota(jnp.int32, (L, L), 0)
        col = jax.lax.broadcasted_iota(jnp.int32, (L, L), 1)

        def seg_rows(base, j, align=SEG):
            r = base + j * SEG
            return r if isinstance(r, int) else pl.multiple_of(r, align)

        def post_attention(j, r0=0, n=SEG, tie=None):
            r = seg_rows(PAD + r0, j, 16)
            av = a_s[pl.ds(r0, n), :]
            if tie is not None:
                av = after(av, tie)
            x1 = (x_s[pl.ds(r, n), :].astype(F32) + mod(2) * av).astype(BF16)
            x_s[pl.ds(r, n), :] = x1
            h2 = (_ln(x1.astype(F32)) * (1.0 + mod(4)) + mod(3)).astype(BF16)
            h_s[pl.ds(r, n), :] = h2
            n2 = _pk(_ln(h2.astype(F32)))
            n2_s[pl.ds(r0 // 2, n // 2), :] = n2
            return n2

        def after(v, dep):
            dep = pltpu.bitcast(dep[:, -LANE:], U32)
            z = dep[:8]
            for r in range(8, dep.shape[0], 8):
                z = z | dep[r:r + 8]
            z = jnp.tile(z & z_s[...], (v.shape[0] // 8, v.shape[1] // LANE))
            return pltpu.bitcast(pltpu.bitcast(v, U32) | z, v.dtype)

        def w1_stage(n2, j):
            r = seg_rows(G0, j)
            for n in range(NCD):
                g = _gelu(_dot(_bf(n2), _bf(w1_s[:, pl.ds(n * LANE, LANE)])))
                g_s[pl.ds(r, SEG), pl.ds(n * LANE, LANE)] = jnp.where(j >= 0, g, 0.0)

        def shifted(j):
            r = seg_rows(G0, j)
            parts = []
            for gi, sh in enumerate((-1, 1, -2, 2)):
                gv = g_s[pl.ds(r - 8, SEG + 16), pl.ds(gi * (D // 4), D // 4)]
                parts.append(gv[8 + sh:8 + sh + SEG].astype(BF16))
            return jnp.concatenate(parts, axis=1)

        def w2_stage(gs, j):
            rp = seg_rows(PAD, j)
            y = h_s[pl.ds(rp, SEG), :].astype(F32) + _dot(gs, _bf(w2_s[...]))
            g_s[pl.ds(seg_rows(G0 - 2 * SEG, j), SEG), :] = x_s[pl.ds(rp, SEG), :].astype(F32) + mod(5) * y
            n = _ln(y)
            hs, hd = SEG // 2, D // 2
            ro = jnp.maximum(j, 0) * (SEG // 4)
            ro = ro if isinstance(j, int) else pl.multiple_of(ro, SEG // 4)
            for i, op in enumerate(_strassen_lhs(n[:hs, :hd], n[:hs, hd:], n[hs:, :hd], n[hs:, hd:])):
                wmod_s[i, pl.ds(ro, SEG // 4), :] = _pk(op)
            return n

        def step(s, carry):
            mask = (row >= SEG) | (col >= SEG) | (row >= col)
            wpos = pl.multiple_of(jax.lax.rem(s * R, RING), 8)
            rpos = pl.multiple_of(jax.lax.rem(s * SEG + OFF, RING), SEG)
            lhs = jnp.concatenate([tok_s[...], lhs_s[...]], axis=0).astype(BF16)

            def proj(j):
                y = _dot(lhs, _bf(wqkv_s[j]))
                ring_s[j, pl.ds(wpos, R), :] = y[:R].astype(BF16)
                return y[R:]

            def full(j, m):
                return jnp.concatenate([ring_s[j, pl.ds(rpos, SEG), :].astype(F32), m], axis=0)

            qs, ks, vs, pr, side = {}, {}, {}, {}, {}
            for i in range(H + LAG_PV):
                if i < H:
                    qm = proj(i)
                    if i in side:
                        qm = after(qm, side.pop(i))
                    if i == CFG['j0']:
                        side[i + CFG['jl']] = post_attention(s - 1, 0, SEG // 2)
                    if i == CFG['j1']:
                        side[i + CFG['jl']] = post_attention(s - 1, SEG // 2, SEG // 2, qm)
                    if i == CFG['j2']:
                        side[i + CFG['jl']] = next_tokens(jnp.minimum(s + 1, NSEG - 1))
                    if i == CFG['j3']:
                        gs = shifted(s - 3)
                        side[i + 2] = pltpu.bitcast(gs, U32)
                if 0 <= i - LAG_QK < H:
                    hq = i - LAG_QK
                    sco = jnp.where(mask, _dot_nt(qs.pop(hq), ks.pop(hq)) * scale, -1e9)
                    e = jnp.exp(sco - jnp.max(sco, axis=-1, keepdims=True))
                    den = jnp.sum(e, axis=-1, keepdims=True)
                    inv = pl.reciprocal(den, approx=True)
                    pr[hq] = e * (inv * (2.0 - den * inv))
                if i < H:
                    km = proj(H + i)
                    qs[i] = full(i, qm)
                    ks[i] = full(H + i, km)
                if 0 <= i - LAG_V < H:
                    hv = i - LAG_V
                    vs[hv] = full(2 * H + hv, proj(2 * H + hv))
                if i == H + LAG_V:
                    ln_y = w2_stage(gs, s - 3)
                if 0 <= i - LAG_PV < H:
                    hp = i - LAG_PV
                    e = pr.pop(hp)
                    o = _dot(e, vs.pop(hp))
                    if CFG['post']:
                        o = o * (1.0 / jnp.sum(e, axis=-1, keepdims=True))
                    o_s[:, pl.ds(hp * LANE, LANE)] = o
            for j in range(NCD):
                ov = o_s[...]
                if j == CFG['j4']:
                    ov = jnp.concatenate([after(ov[:, :LANE], ln_y), ov[:, LANE:]], axis=1)
                y = _dot(ov, _bf(wo_s[:, pl.ds(j * LANE, LANE)]))
                a_s[:, pl.ds(j * LANE, LANE)] = y[:SEG]
                lhs_s[:, pl.ds(j * LANE, LANE)] = y[SEG:]
            w1_stage(n2_s[...], s - 1)
            return carry

        _loop('steps', NSEG, step, CFG['us'])
        n2 = post_attention(NSEG - 1)
        w2_stage(shifted(NSEG - 3), NSEG - 3)
        w1_stage(n2, NSEG - 1)
        w2_stage(shifted(NSEG - 2), NSEG - 2)
        w2_stage(shifted(NSEG - 1), NSEG - 1)

        for cp in cp_w3 + cp_w4:
            cp.wait()

        NT = F // 2 // LANE
        HS = S // 2

        def u_op(i, t):
            if i < 6:
                return wqkv_s.at[i * 16 + t]
            return u7_s.at[t]

        def rhs_sums(w, n1, n2, kh):
            b11, b12 = w.at[n1, pl.ds(0, kh)], w.at[n2, pl.ds(0, kh)]
            b21, b22 = w.at[n1, pl.ds(kh, kh)], w.at[n2, pl.ds(kh, kh)]
            for r in range(0, kh, 32):
                rows = pl.ds(r, 32)
                v11, v12, v21, v22 = (_bf(b[rows, :]).astype(F32) for b in (b11, b12, b21, b22))
                for i, v in enumerate((v11 + v22, v12 - v22, v21 - v11, v11 + v12, v21 + v22)):
                    ws_s[i, rows, :] = _pk(v)
            sm = [ws_s.at[i, pl.ds(0, kh)] for i in range(5)]
            return [sm[0], b11, sm[1], sm[2], b22, sm[3], sm[4]]

        def mlp1(t, carry):
            b = rhs_sums(w3_s, t, NT + t, D // 4)
            RB = CFG['rb1']
            for r in range(0, HS, RB):
                rows = pl.ds(r // 2, RB // 2)
                c = _strassen(lambda i: _dot(_bf(wmod_s[i, rows, :]), _bf(b[i][...])))
                for i, op in enumerate(_strassen_lhs(*map(_gelu, c))):
                    u_op(i, t)[rows, :] = _pk(op)
            return carry
        _loop('mlp1', NT, mlp1, CFG['um'])

        NH = NCD // 2
        BM = CFG['bm']
        osem = next(sem_i)

        def out_copy(it, half):
            rows = pl.ds(pl.multiple_of((it // NH) * BM, BM), BM)
            cols = pl.ds(pl.multiple_of((it % NH + half * NH) * LANE, LANE), LANE)
            slot = (it % 2) * 2 + half
            return pltpu.make_async_copy(ob_s.at[slot], out_hbm.at[rows, cols], sems.at[osem + slot])

        def mlp2(it, carry):
            @pl.when(it > 1)
            def _():
                out_copy(it - 2, 0).wait()
                out_copy(it - 2, 1).wait()
            blk, n = it // NH, it % NH
            b = rhs_sums(w4_s, n, NH + n, F // 4)
            RB = CFG['rb2']
            for r in range(0, BM // 2, RB):
                rows = pl.ds(pl.multiple_of(blk * (BM // 4) + r // 2, RB // 2), RB // 2)

                def prod(i):
                    lhs = jnp.concatenate([_bf(u_op(i, t)[rows, :]) for t in range(NT)], axis=1)
                    return _dot(lhs, _bf(b[i][...]))
                c11, c12, c21, c22 = _strassen(prod)
                for half, (ct, cb) in enumerate(((c11, c21), (c12, c22))):
                    cols = pl.ds(pl.multiple_of((n + half * NH) * LANE, LANE), LANE)
                    hs = SEG // 2
                    y = jnp.concatenate([v[q:q + hs] for q in range(0, RB, hs) for v in (ct, cb)], axis=0)
                    base = g_s[pl.ds(pl.multiple_of(G0 - 2 * SEG + blk * BM + 2 * r, SEG), 2 * RB), cols]
                    ob_s[(it % 2) * 2 + half, pl.ds(2 * r, 2 * RB), :] = (base + gb_s[n + half * NH, pl.ds(0, 1), :] * y).astype(BF16)
            out_copy(it, 0).start()
            out_copy(it, 1).start()
            return carry
        for n in range(NCD):
            gb_s[n] = jnp.broadcast_to(mod(5)[:, n * LANE:(n + 1) * LANE], (8, LANE))
        nit = (S // BM) * NH
        _loop('mlp2', nit, mlp2)
        for it in (nit - 2, nit - 1):
            out_copy(it, 0).wait()
            out_copy(it, 1).wait()

    scratch = [
        pltpu.VMEM((PAD + S, D), BF16),
        pltpu.VMEM((PAD + S, D), BF16),
        pltpu.VMEM((NKB, P // 2, DK), U32),
        pltpu.VMEM((3 * H, D // 2, LANE), U32),
        pltpu.VMEM((H * LANE // 2, D), U32),
        pltpu.VMEM((D // 2, D), U32),
        pltpu.VMEM((D // 2, D), U32),
        pltpu.VMEM((F // LANE, D // 2, LANE), U32),
        pltpu.VMEM((NCD, F // 2, LANE), U32),
        pltpu.VMEM((6 * D // MP, D // 2, MP), U32),
        pltpu.VMEM((NST, DK, H // 2, LANE), U32),
        pltpu.VMEM((3 * H, RING, LANE), BF16),
        pltpu.VMEM((6 * D // MP, 8, MP), F32),
        pltpu.VMEM((R, D), F32),
        pltpu.VMEM((M, D), F32),
        pltpu.VMEM((L, H * LANE), F32),
        pltpu.VMEM((SEG, D), F32),
        pltpu.VMEM((SEG // 2, D), U32),
        pltpu.VMEM((G0 + S + 8, D), F32),
        pltpu.VMEM((NKB, P, DK), F32),
        pltpu.VMEM((5, F // 4, LANE), U32),
        pltpu.VMEM((F // 2 // LANE, S // 4, LANE), U32),
        pltpu.VMEM((NCD, 8, LANE), F32),
        pltpu.VMEM((4, CFG['bm'], LANE), BF16),
        pltpu.VMEM((8, LANE), U32),
        pltpu.VMEM((592, LANE), U32),
        pltpu.SemaphoreType.DMA((64,)),
        pltpu.SemaphoreType.DMA((NST * NSUB,)),
        pltpu.SemaphoreType.DMA((12 * D // MP,)),
    ]
    return kernel, scratch


@functools.partial(jax.jit, static_argnames=("A_seg_len",))
def pallas_adaLN_cond__memory_aug_recurrent_mem_tr__mixer_s_mlp__prompt_kernel(
    A_x: jax.Array,
    A_mem0: jax.Array,
    A_Wq: jax.Array,
    A_Wk: jax.Array,
    A_Wv: jax.Array,
    A_Wo: jax.Array,
    A_seg_len: int,
    B_x: jax.Array,
    B_w1: jax.Array,
    B_w2: jax.Array,
    B_w3: jax.Array,
    B_w4: jax.Array,
    c: jax.Array,
    w_mod: jax.Array,
):
    del B_x
    B, S, D = A_x.shape
    _, H, Dh = A_Wq.shape
    M = A_mem0.shape[1]
    F = B_w3.shape[1]
    assert B == 1 and Dh == LANE
    kernel, scratch = _make_kernel(S, D, H, M, int(A_seg_len), F)
    hbm = pl.BlockSpec(memory_space=pl.ANY)
    vmem = pl.BlockSpec(memory_space=pltpu.VMEM)
    out = pl.pallas_call(
        kernel,
        in_specs=[hbm, vmem, hbm, hbm, hbm, hbm, hbm, hbm, hbm, hbm, vmem, hbm],
        out_specs=hbm,
        out_shape=jax.ShapeDtypeStruct((S, D), A_x.dtype),
        scratch_shapes=scratch,
        compiler_params=pltpu.CompilerParams(vmem_limit_bytes=127 * 1024 * 1024, flags={0: None, 1: {'XLA_TPU_FORCE_LP_LLO_SCHEDULER': True}, 2: {'XLA_TPU_EVENLY_DISTRIBUTE_CRITICAL_NODES': True}}[CFG['fl']]),
    )(A_x.reshape(S, D), A_mem0.reshape(M, D), A_Wq, A_Wk, A_Wv, A_Wo.reshape(H * Dh, D),
      B_w1, B_w2, B_w3, B_w4, c, w_mod)
    return out.reshape(B, S, D)
```

```python
import contextlib
import functools

import jax
import jax.numpy as jnp
import numpy as np
import jax.experimental.pallas as pl
import jax.experimental.pallas.tpu as pltpu

F32 = jnp.float32
BF16 = jnp.bfloat16
U32 = jnp.uint32
LANE = 128
CFG = dict(qk=2, v=3, pv=5, post=0, rb=128, fl=2, tie=1, prof=0, us=2, um=2, nsub=1, j0=0, j1=7, j2=14, j3=22, jl=6, j4=3, w1=8, rb1=128, rb2=512, bm=1024)


def _scope(n):
    return jax.named_scope(n) if CFG['prof'] else contextlib.nullcontext()


def _loop(name, n, body, unroll=1):
    def group(i, carry):
        for u in range(unroll):
            body(i * unroll + u, carry)
        return carry
    with _scope(name):
        jax.lax.fori_loop(0, n // unroll, group, 0)


def _dot(a, b):
    return jax.lax.dot_general(a, b, (((1,), (0,)), ((), ())), preferred_element_type=F32)


def _dot_nt(a, b):
    return jax.lax.dot_general(a, b, (((1,), (1,)), ((), ())), preferred_element_type=F32)


def _bf(w):
    return pltpu.bitcast(w, BF16)


def _pk(x):
    return pltpu.bitcast(x.astype(BF16), U32)


def _ln(x):
    m = jnp.mean(x, axis=-1, keepdims=True)
    xc = x - m
    v = jnp.mean(xc * xc, axis=-1, keepdims=True)
    return xc * jax.lax.rsqrt(v + 1e-5)


def _gelu(x):
    return jax.nn.gelu(x, approximate=True)


def _strassen_lhs(a11, a12, a21, a22):
    return a11 + a22, a21 + a22, a11, a22, a11 + a12, a21 - a11, a12 - a22


def _strassen(prod):
    m2 = prod(1)
    m5 = prod(4)
    m4 = prod(3)
    c21 = m2 + m4
    c11 = m4 - m5
    m3 = prod(2)
    c12 = m3 + m5
    c22 = m3 - m2
    m1 = prod(0)
    c11 = c11 + m1
    c22 = c22 + m1
    c11 = c11 + prod(6)
    c22 = c22 + prod(5)
    return c11, c12, c21, c22


def _make_kernel(S, D, H, M, SEG, F):
    NSEG = S // SEG
    R = SEG - M
    P = S - R * NSEG
    RING = 576
    OFF = RING - P
    L = SEG + M
    NCD = D // LANE
    PAD = 3 * SEG
    G0 = 5 * SEG
    LAG_QK, LAG_V, LAG_PV = CFG['qk'], CFG['v'], CFG['pv']
    scale = float(LANE) ** -0.5

    DK = 2 * LANE
    NKB = D // DK
    NPC = 3 * NKB
    NSUB = CFG['nsub']
    NST = 4
    MP = 2 * DK

    def kernel(x_hbm, mem0_ref, wq_hbm, wk_hbm, wv_hbm, wo_hbm, w1_hbm, w2_hbm, w3_hbm, w4_hbm, c_ref, wmod_hbm,
               out_hbm,
               x_s, h_s, h0_s, wqkv_s, wo_s, w1_s, w2_s, w3_s, w4_s, wmod_s, stage_s, ring_s, mod_s, tok_s, lhs_s,
               o_s, a_s, n2_s, g_s, n0_s, ws_s, u7_s, gb_s, ob_s, z_s, t_s, sems, wsems, msems):
        sem_i = iter(range(64))

        def copy(src, dst):
            return pltpu.make_async_copy(src, dst, sems.at[next(sem_i)])

        def cp_w(pc, q, w=wq_hbm):
            n = DK // NSUB
            src = w.at[pl.ds((pc % NKB) * DK + q * n, n)]
            dst = stage_s.at[pc % NST, pl.ds(q * n, n)].bitcast(BF16)
            return pltpu.make_async_copy(src, dst, wsems.at[(pc % NST) * NSUB + q])

        def cp_mod(j, q):
            col = jnp.where(j < NKB, q * D + j * DK, j * MP + q * DK)
            src = wmod_hbm.at[:, pl.ds(pl.multiple_of(col, DK), DK)]
            return pltpu.make_async_copy(src, wmod_s.at[j, :, pl.ds(q * DK, DK)].bitcast(BF16), msems.at[2 * j + q])

        def start_piece(pc):
            for t, w in enumerate((wq_hbm, wk_hbm, wv_hbm)):
                @pl.when(pc // NKB == t)
                def _():
                    for q in range(NSUB):
                        cp_w(pc, q, w).start()

        def start_mod(j):
            cp_mod(j, 0).start()
            cp_mod(j, 1).start()

        cp_x0 = copy(x_hbm.at[pl.ds(0, P)], x_s.at[pl.ds(PAD, P)])
        NWO = 8
        wo_sem = [next(sem_i) for _ in range(NWO)][0]

        def cp_wo(j):
            n = H * LANE // NWO
            src = wo_hbm.at[pl.ds(pl.multiple_of(j * n, n), n)]
            dst = wo_s.at[pl.ds(pl.multiple_of(j * (n // 2), n // 2), n // 2)].bitcast(BF16)
            return pltpu.make_async_copy(src, dst, sems.at[wo_sem + j])

        late = [copy(w1_hbm, w1_s.bitcast(BF16)), copy(x_hbm.at[pl.ds(P, S - P)], x_s.at[pl.ds(PAD + P, S - P)]),
                copy(w2_hbm, w2_s.bitcast(BF16))]
        cp_w3 = [copy(w3_hbm.at[:, pl.ds(j * LANE, LANE)], w3_s.at[j].bitcast(BF16)) for j in range(F // LANE)]
        cp_w4 = [copy(w4_hbm.at[:, pl.ds(j * LANE, LANE)], w4_s.at[j].bitcast(BF16)) for j in range(NCD)]

        cp_x0.start()
        for q in range(NSUB):
            cp_w(0, q).start()
        start_mod(0)

        cv = jnp.broadcast_to(c_ref[...].astype(F32), (8, D))
        sc = cv * jax.nn.sigmoid(cv)

        def mod(i):
            if i < 2:
                return jnp.concatenate([mod_s[j, pl.ds(0, 1), pl.ds(i * DK, DK)] for j in range(NKB)], axis=1)
            n = D // MP
            return jnp.concatenate([mod_s[i * n + j, pl.ds(0, 1), :] for j in range(n)], axis=1)

        x_s[pl.ds(0, PAD), :] = jnp.zeros((PAD, D), BF16)
        h_s[pl.ds(0, PAD), :] = jnp.zeros((PAD, D), BF16)
        a_s[...] = jnp.zeros(a_s.shape, F32)
        z_s[...] = jnp.zeros(z_s.shape, U32)
        g_s[pl.ds(0, G0), :] = jnp.zeros((G0, D), F32)
        g_s[pl.ds(G0 + S, 8), :] = jnp.zeros((8, D), F32)

        def relayout(pc, u, tie=None):
            d0, hg = (u // 2) * 16, u % 2
            v = stage_s[pc % NST, pl.ds(d0, 16), pl.ds(hg * 8, 8), :]
            if tie is not None:
                v = v | tie[None]
            v = v.reshape(8, 2, 8, LANE)
            a, b = v[:, 0], v[:, 1]
            lo = (a & 0xFFFF) | (b << 16)
            hi = (a >> 16) | (b & np.uint32(0xFFFF0000))
            t0 = (u % 4) * 144
            for q in range(8):
                t_s[pl.ds(t0 + q * 9, 8), :] = lo[q]
                t_s[pl.ds(t0 + 72 + q * 9, 8), :] = hi[q]
            rows = pl.ds(pl.multiple_of((pc % NKB) * (DK // 2) + d0 // 2, 8), 8)
            head = (pc // NKB) * H + hg * 16
            for j in range(8):
                wqkv_s[head + 2 * j, rows, :] = t_s[pl.ds(t0 + j, 8, stride=9), :]
                wqkv_s[head + 2 * j + 1, rows, :] = t_s[pl.ds(t0 + 72 + j, 8, stride=9), :]

        NU = DK // 16 * 2

        def mod_cols(j, b):
            cols = pl.ds(b * LANE, LANE)
            mod_s[j, :, cols] = _dot(sc, _bf(wmod_s[j, :, cols]))

        def modulate(j):
            cp_mod(j, 0).wait()
            cp_mod(j, 1).wait()
            for b in range(MP // LANE):
                mod_cols(j, b)
            m = mod_s[j, pl.ds(0, 1), :]
            for r in range(0, P, 64):
                hv = n0_s[j, pl.ds(r, 64), :] * (1.0 + m[:, DK:]) + m[:, :DK]
                h0_s[j, pl.ds(r // 2, 32), :] = _pk(hv)

        cp_x0.wait()

        def ln0(i, carry):
            r = pl.multiple_of(i * 128, 128)
            n = _ln(x_s[pl.ds(pl.multiple_of(PAD + r, 32), 128), :].astype(F32))
            for j in range(NKB):
                n0_s[j, pl.ds(r, 128), :] = n[:, j * DK:(j + 1) * DK]
            return carry
        _loop('ln0', P // 128, ln0)

        def bulk(pc, carry):
            @pl.when(pc < 2)
            def _():
                cp_w(pc, 0).wait()
                for u in range(NU):
                    relayout(pc, u)
            pl.when(pc < NKB)(lambda: modulate(pc))
            more = (pc > 0) & (pc + 1 < NPC)
            nxt = jnp.where(more, pc + 1, pc)
            pl.when(more)(cp_w(nxt, 0).wait)
            for q in range(2):
                pl.when(pc >= NKB)(cp_mod(pc, q).wait)
            pl.when(pc == 0)(cp_w(1, 0).start)
            pl.when(pc + 1 < NPC)(lambda: start_mod(pc + 1))
            start_piece(pc + 2)
            pl.when((pc > 0) & (pc <= NWO))(lambda: cp_wo(pc - 1).start())
            for i, cp in enumerate(late):
                pl.when(pc == NPC - len(late) + i)(cp.start)

            kb = pc % NKB
            rows = pl.ds(pl.multiple_of(kb * (DK // 2), DK // 2), DK // 2)
            RB = CFG['rb']
            for hd in range(H):
                j = (pc // NKB) * H + hd
                for r in range(0, P, RB):
                    acc = g_s.at[pl.ds(G0 + (hd // NCD) * P + r, RB), pl.ds((hd % NCD) * LANE, LANE)]
                    y = _dot(_bf(h0_s[kb, pl.ds(r // 2, RB // 2), :]), _bf(wqkv_s[j, rows, :]))
                    if r == 0:
                        tie = pltpu.bitcast(y[:8], U32) & z_s[...]
                    y = y + jnp.where(kb > 0, acc[...], 0.0)
                    acc[...] = y
                    ring_s[j, pl.ds(OFF + r, RB), :] = y.astype(BF16)
                relayout(nxt, hd, tie)
                if hd % 8 == 4:
                    mod_cols(pc, hd // 8)
            return carry
        _loop('bulk', NPC, bulk)

        with _scope('late'):
            for cp in late + [cp_wo(j) for j in range(NWO)]:
                cp.wait()
        for cp in cp_w3 + cp_w4:
            cp.start()

        def next_tokens(s):
            r = PAD + P + s * R
            xv = x_s[pl.ds(r if isinstance(r, int) else pl.multiple_of(r, 8), R), :].astype(F32)
            t = _ln(xv) * (1.0 + mod(1)) + mod(0)
            tok_s[...] = t
            return t

        next_tokens(0)
        lhs_s[...] = mem0_ref[...].astype(F32)

        row = jax.lax.broadcasted_iota(jnp.int32, (L, L), 0)
        col = jax.lax.broadcasted_iota(jnp.int32, (L, L), 1)

        def seg_rows(base, j, align=SEG):
            r = base + j * SEG
            return r if isinstance(r, int) else pl.multiple_of(r, align)

        def post_attention(j, r0=0, n=SEG, tie=None):
            r = seg_rows(PAD + r0, j, 16)
            av = a_s[pl.ds(r0, n), :]
            if tie is not None:
                av = after(av, tie)
            x1 = (x_s[pl.ds(r, n), :].astype(F32) + mod(2) * av).astype(BF16)
            x_s[pl.ds(r, n), :] = x1
            h2 = (_ln(x1.astype(F32)) * (1.0 + mod(4)) + mod(3)).astype(BF16)
            h_s[pl.ds(r, n), :] = h2
            n2 = _pk(_ln(h2.astype(F32)))
            n2_s[pl.ds(r0 // 2, n // 2), :] = n2
            return n2

        def after(v, dep):
            dep = pltpu.bitcast(dep[:, -LANE:], U32)
            z = dep[:8]
            for r in range(8, dep.shape[0], 8):
                z = z | dep[r:r + 8]
            z = jnp.tile(z & z_s[...], (v.shape[0] // 8, v.shape[1] // LANE))
            return pltpu.bitcast(pltpu.bitcast(v, U32) | z, v.dtype)

        def w1_stage(n2, j):
            r = seg_rows(G0, j)
            for n in range(NCD):
                g = _gelu(_dot(_bf(n2), _bf(w1_s[:, pl.ds(n * LANE, LANE)])))
                g_s[pl.ds(r, SEG), pl.ds(n * LANE, LANE)] = jnp.where(j >= 0, g, 0.0)

        def shifted(j):
            r = seg_rows(G0, j)
            parts = []
            for gi, sh in enumerate((-1, 1, -2, 2)):
                gv = g_s[pl.ds(r - 8, SEG + 16), pl.ds(gi * (D // 4), D // 4)]
                parts.append(gv[8 + sh:8 + sh + SEG].astype(BF16))
            return jnp.concatenate(parts, axis=1)

        def w2_stage(gs, j):
            rp = seg_rows(PAD, j)
            y = h_s[pl.ds(rp, SEG), :].astype(F32) + _dot(gs, _bf(w2_s[...]))
            g_s[pl.ds(seg_rows(G0 - 2 * SEG, j), SEG), :] = x_s[pl.ds(rp, SEG), :].astype(F32) + mod(5) * y
            n = _ln(y)
            hs, hd = SEG // 2, D // 2
            ro = jnp.maximum(j, 0) * (SEG // 4)
            ro = ro if isinstance(j, int) else pl.multiple_of(ro, SEG // 4)
            for i, op in enumerate(_strassen_lhs(n[:hs, :hd], n[:hs, hd:], n[hs:, :hd], n[hs:, hd:])):
                wmod_s[i, pl.ds(ro, SEG // 4), :] = _pk(op)
            return n

        def step(s, carry):
            mask = (row >= SEG) | (col >= SEG) | (row >= col)
            wpos = pl.multiple_of(jax.lax.rem(s * R, RING), 8)
            rpos = pl.multiple_of(jax.lax.rem(s * SEG + OFF, RING), SEG)
            lhs = jnp.concatenate([tok_s[...], lhs_s[...]], axis=0).astype(BF16)

            def proj(j):
                y = _dot(lhs, _bf(wqkv_s[j]))
                ring_s[j, pl.ds(wpos, R), :] = y[:R].astype(BF16)
                return y[R:]

            def full(j, m):
                return jnp.concatenate([ring_s[j, pl.ds(rpos, SEG), :].astype(F32), m], axis=0)

            qs, ks, vs, pr, side = {}, {}, {}, {}, {}
            for i in range(H + LAG_PV):
                if i < H:
                    qm = proj(i)
                    if i in side:
                        qm = after(qm, side.pop(i))
                    if i == CFG['j0']:
                        side[i + CFG['jl']] = post_attention(s - 1, 0, SEG // 2)
                    if i == CFG['j1']:
                        side[i + CFG['jl']] = post_attention(s - 1, SEG // 2, SEG // 2, qm)
                    if i == CFG['j2']:
                        side[i + CFG['jl']] = next_tokens(jnp.minimum(s + 1, NSEG - 1))
                    if i == CFG['j3']:
                        gs = shifted(s - 3)
                        side[i + 2] = pltpu.bitcast(gs, U32)
                if 0 <= i - LAG_QK < H:
                    hq = i - LAG_QK
                    sco = jnp.where(mask, _dot_nt(qs.pop(hq), ks.pop(hq)) * scale, -1e9)
                    e = jnp.exp(sco - jnp.max(sco, axis=-1, keepdims=True))
                    den = jnp.sum(e, axis=-1, keepdims=True)
                    inv = pl.reciprocal(den, approx=True)
                    pr[hq] = e * (inv * (2.0 - den * inv))
                if i < H:
                    km = proj(H + i)
                    qs[i] = full(i, qm)
                    ks[i] = full(H + i, km)
                if 0 <= i - LAG_V < H:
                    hv = i - LAG_V
                    vs[hv] = full(2 * H + hv, proj(2 * H + hv))
                if i == H + LAG_V:
                    ln_y = w2_stage(gs, s - 3)
                if 0 <= i - LAG_PV < H:
                    hp = i - LAG_PV
                    e = pr.pop(hp)
                    o = _dot(e, vs.pop(hp))
                    if CFG['post']:
                        o = o * (1.0 / jnp.sum(e, axis=-1, keepdims=True))
                    o_s[:, pl.ds(hp * LANE, LANE)] = o
            for j in range(NCD):
                ov = o_s[...]
                if j == CFG['j4']:
                    ov = jnp.concatenate([after(ov[:, :LANE], ln_y), ov[:, LANE:]], axis=1)
                y = _dot(ov, _bf(wo_s[:, pl.ds(j * LANE, LANE)]))
                a_s[:, pl.ds(j * LANE, LANE)] = y[:SEG]
                lhs_s[:, pl.ds(j * LANE, LANE)] = y[SEG:]
            w1_stage(n2_s[...], s - 1)
            return carry

        _loop('steps', NSEG, step, CFG['us'])
        n2 = post_attention(NSEG - 1)
        w2_stage(shifted(NSEG - 3), NSEG - 3)
        w1_stage(n2, NSEG - 1)
        w2_stage(shifted(NSEG - 2), NSEG - 2)
        w2_stage(shifted(NSEG - 1), NSEG - 1)

        for cp in cp_w3 + cp_w4:
            cp.wait()

        NT = F // 2 // LANE
        HS = S // 2

        def u_op(i, t):
            if i < 6:
                return wqkv_s.at[i * 16 + t]
            return u7_s.at[t]

        def rhs_sums(w, n1, n2, kh):
            b11, b12 = w.at[n1, pl.ds(0, kh)], w.at[n2, pl.ds(0, kh)]
            b21, b22 = w.at[n1, pl.ds(kh, kh)], w.at[n2, pl.ds(kh, kh)]
            for r in range(0, kh, 32):
                rows = pl.ds(r, 32)
                v11, v12, v21, v22 = (_bf(b[rows, :]).astype(F32) for b in (b11, b12, b21, b22))
                for i, v in enumerate((v11 + v22, v12 - v22, v21 - v11, v11 + v12, v21 + v22)):
                    ws_s[i, rows, :] = _pk(v)
            sm = [ws_s.at[i, pl.ds(0, kh)] for i in range(5)]
            return [sm[0], b11, sm[1], sm[2], b22, sm[3], sm[4]]

        def mlp1(t, carry):
            b = rhs_sums(w3_s, t, NT + t, D // 4)
            RB = CFG['rb1']
            for r in range(0, HS, RB):
                rows = pl.ds(r // 2, RB // 2)
                c = _strassen(lambda i: _dot(_bf(wmod_s[i, rows, :]), _bf(b[i][...])))
                for i, op in enumerate(_strassen_lhs(*map(_gelu, c))):
                    u_op(i, t)[rows, :] = _pk(op)
            return carry
        _loop('mlp1', NT, mlp1, CFG['um'])

        NH = NCD // 2
        BM = CFG['bm']
        osem = next(sem_i)

        def out_copy(it, half):
            rows = pl.ds(pl.multiple_of((it // NH) * BM, BM), BM)
            cols = pl.ds(pl.multiple_of((it % NH + half * NH) * LANE, LANE), LANE)
            slot = (it % 2) * 2 + half
            return pltpu.make_async_copy(ob_s.at[slot], out_hbm.at[rows, cols], sems.at[osem + slot])

        def mlp2(it, carry):
            @pl.when(it > 1)
            def _():
                out_copy(it - 2, 0).wait()
                out_copy(it - 2, 1).wait()
            blk, n = it // NH, it % NH
            b = rhs_sums(w4_s, n, NH + n, F // 4)
            RB = CFG['rb2']
            for r in range(0, BM // 2, RB):
                rows = pl.ds(pl.multiple_of(blk * (BM // 4) + r // 2, RB // 2), RB // 2)

                def prod(i):
                    lhs = jnp.concatenate([_bf(u_op(i, t)[rows, :]) for t in range(NT)], axis=1)
                    return _dot(lhs, _bf(b[i][...]))
                c11, c12, c21, c22 = _strassen(prod)
                for half, (ct, cb) in enumerate(((c11, c21), (c12, c22))):
                    cols = pl.ds(pl.multiple_of((n + half * NH) * LANE, LANE), LANE)
                    hs = SEG // 2
                    y = jnp.concatenate([v[q:q + hs] for q in range(0, RB, hs) for v in (ct, cb)], axis=0)
                    base = g_s[pl.ds(pl.multiple_of(G0 - 2 * SEG + blk * BM + 2 * r, SEG), 2 * RB), cols]
                    ob_s[(it % 2) * 2 + half, pl.ds(2 * r, 2 * RB), :] = (base + gb_s[n + half * NH, pl.ds(0, 1), :] * y).astype(BF16)
            out_copy(it, 0).start()
            out_copy(it, 1).start()
            return carry
        for n in range(NCD):
            gb_s[n] = jnp.broadcast_to(mod(5)[:, n * LANE:(n + 1) * LANE], (8, LANE))
        nit = (S // BM) * NH
        _loop('mlp2', nit, mlp2)
        for it in (nit - 2, nit - 1):
            out_copy(it, 0).wait()
            out_copy(it, 1).wait()

    scratch = [
        pltpu.VMEM((PAD + S, D), BF16),
        pltpu.VMEM((PAD + S, D), BF16),
        pltpu.VMEM((NKB, P // 2, DK), U32),
        pltpu.VMEM((3 * H, D // 2, LANE), U32),
        pltpu.VMEM((H * LANE // 2, D), U32),
        pltpu.VMEM((D // 2, D), U32),
        pltpu.VMEM((D // 2, D), U32),
        pltpu.VMEM((F // LANE, D // 2, LANE), U32),
        pltpu.VMEM((NCD, F // 2, LANE), U32),
        pltpu.VMEM((6 * D // MP, D // 2, MP), U32),
        pltpu.VMEM((NST, DK, H // 2, LANE), U32),
        pltpu.VMEM((3 * H, RING, LANE), BF16),
        pltpu.VMEM((6 * D // MP, 8, MP), F32),
        pltpu.VMEM((R, D), F32),
        pltpu.VMEM((M, D), F32),
        pltpu.VMEM((L, H * LANE), F32),
        pltpu.VMEM((SEG, D), F32),
        pltpu.VMEM((SEG // 2, D), U32),
        pltpu.VMEM((G0 + S + 8, D), F32),
        pltpu.VMEM((NKB, P, DK), F32),
        pltpu.VMEM((5, F // 4, LANE), U32),
        pltpu.VMEM((F // 2 // LANE, S // 4, LANE), U32),
        pltpu.VMEM((NCD, 8, LANE), F32),
        pltpu.VMEM((4, CFG['bm'], LANE), BF16),
        pltpu.VMEM((8, LANE), U32),
        pltpu.VMEM((592, LANE), U32),
        pltpu.SemaphoreType.DMA((64,)),
        pltpu.SemaphoreType.DMA((NST * NSUB,)),
        pltpu.SemaphoreType.DMA((12 * D // MP,)),
    ]
    return kernel, scratch


@functools.partial(jax.jit, static_argnames=("A_seg_len",))
def pallas_adaLN_cond__memory_aug_recurrent_mem_tr__mixer_s_mlp__prompt_kernel(
    A_x: jax.Array,
    A_mem0: jax.Array,
    A_Wq: jax.Array,
    A_Wk: jax.Array,
    A_Wv: jax.Array,
    A_Wo: jax.Array,
    A_seg_len: int,
    B_x: jax.Array,
    B_w1: jax.Array,
    B_w2: jax.Array,
    B_w3: jax.Array,
    B_w4: jax.Array,
    c: jax.Array,
    w_mod: jax.Array,
):
    del B_x
    B, S, D = A_x.shape
    _, H, Dh = A_Wq.shape
    M = A_mem0.shape[1]
    F = B_w3.shape[1]
    assert B == 1 and Dh == LANE
    kernel, scratch = _make_kernel(S, D, H, M, int(A_seg_len), F)
    hbm = pl.BlockSpec(memory_space=pl.ANY)
    vmem = pl.BlockSpec(memory_space=pltpu.VMEM)
    out = pl.pallas_call(
        kernel,
        in_specs=[hbm, vmem, hbm, hbm, hbm, hbm, hbm, hbm, hbm, hbm, vmem, hbm],
        out_specs=hbm,
        out_shape=jax.ShapeDtypeStruct((S, D), A_x.dtype),
        scratch_shapes=scratch,
        compiler_params=pltpu.CompilerParams(vmem_limit_bytes=127 * 1024 * 1024, flags={0: None, 1: {'XLA_TPU_FORCE_LP_LLO_SCHEDULER': True}, 2: {'XLA_TPU_EVENLY_DISTRIBUTE_CRITICAL_NODES': True}}[CFG['fl']]),
    )(A_x.reshape(S, D), A_mem0.reshape(M, D), A_Wq, A_Wk, A_Wv, A_Wo.reshape(H * Dh, D),
      B_w1, B_w2, B_w3, B_w4, c, w_mod)
    return out.reshape(B, S, D)
```

```python
import functools

import jax
import jax.numpy as jnp
import numpy as np
import jax.experimental.pallas as pl
import jax.experimental.pallas.tpu as pltpu

F32 = jnp.float32
BF16 = jnp.bfloat16
U32 = jnp.uint32
LANE = 128


def _dot(a, b):
    return jax.lax.dot_general(a, b, (((1,), (0,)), ((), ())), preferred_element_type=F32)


def _dot_nt(a, b):
    return jax.lax.dot_general(a, b, (((1,), (1,)), ((), ())), preferred_element_type=F32)


def _bf(w):
    return pltpu.bitcast(w, BF16)


def _pk(x):
    return pltpu.bitcast(x.astype(BF16), U32)


def _ln(x):
    m = jnp.mean(x, axis=-1, keepdims=True)
    xc = x - m
    v = jnp.mean(xc * xc, axis=-1, keepdims=True)
    return xc * jax.lax.rsqrt(v + 1e-5)


def _gelu(x):
    return jax.nn.gelu(x, approximate=True)


def _strassen_lhs(a11, a12, a21, a22):
    return a11 + a22, a21 + a22, a11, a22, a11 + a12, a21 - a11, a12 - a22


def _strassen_rhs_sums(b11, b12, b21, b22):
    return b11 + b22, b12 - b22, b21 - b11, b11 + b12, b21 + b22


def _strassen(prod):
    m2 = prod(1)
    m5 = prod(4)
    m4 = prod(3)
    c21 = m2 + m4
    c11 = m4 - m5
    m3 = prod(2)
    c12 = m3 + m5
    c22 = m3 - m2
    m1 = prod(0)
    c11 = c11 + m1
    c22 = c22 + m1
    c11 = c11 + prod(6)
    c22 = c22 + prod(5)
    return c11, c12, c21, c22


def _loop(n, body, unroll=1):
    def group(i, carry):
        for u in range(unroll):
            body(i * unroll + u)
        return carry
    jax.lax.fori_loop(0, n // unroll, group, 0)


def _make_kernel(S, D, H, M, SEG, F):
    NSEG = S // SEG
    L = SEG + M
    R = SEG - M
    P = S - R * NSEG
    RING = P + 2 * SEG
    OFF = RING - P
    NCD = D // LANE
    LAG_W2 = 3
    PAD = LAG_W2 * SEG
    G0 = PAD + 2 * SEG
    LAG_QK, LAG_V, LAG_PV = 3, 3, 6
    DK = 2 * LANE
    NKB = D // DK
    NPC = 3 * NKB
    NST = 4
    NU = 2 * DK // 16
    MP = 2 * DK
    NWO = 8
    NT = F // 2 // LANE
    NH = NCD // 2
    BM = S // 2
    assert RING % R == 0 and RING % SEG == 0 and OFF % SEG == 0 and NU == H and 6 * D // MP == NPC
    scale = float(LANE) ** -0.5

    def kernel(x_hbm, mem0_ref, wq_hbm, wk_hbm, wv_hbm, wo_hbm, w1_hbm, w2_hbm, w3_hbm, w4_hbm, c_ref, wmod_hbm,
               out_hbm,
               x_s, h_s, h0_s, wqkv_s, wo_s, w1_s, w2_s, w3_s, w4_s, wmod_s, stage_s, ring_s, mod_s, tok_s, mem_s,
               o_s, a_s, n2_s, g_s, n0_s, ws_s, u7_s, gb_s, ob_s, z_s, t_s,
               sems, w_sems, m_sems, wo_sems, o_sems):
        sem_i = iter(range(sems.shape[0]))

        def copy(src, dst):
            return pltpu.make_async_copy(src, dst, sems.at[next(sem_i)])

        def cp_w(pc, w=wq_hbm):
            return pltpu.make_async_copy(w.at[pl.ds((pc % NKB) * DK, DK)], stage_s.at[pc % NST].bitcast(BF16),
                                         w_sems.at[pc % NST])

        def start_piece(pc):
            for t, w in enumerate((wq_hbm, wk_hbm, wv_hbm)):
                pl.when(pc // NKB == t)(lambda w=w: cp_w(pc, w).start())

        def cp_mod(j, q):
            col = jnp.where(j < NKB, q * D + j * DK, j * MP + q * DK)
            src = wmod_hbm.at[:, pl.ds(pl.multiple_of(col, DK), DK)]
            return pltpu.make_async_copy(src, wmod_s.at[j, :, pl.ds(q * DK, DK)].bitcast(BF16), m_sems.at[2 * j + q])

        def start_mod(j):
            cp_mod(j, 0).start()
            cp_mod(j, 1).start()

        def wait_mod(j):
            cp_mod(j, 0).wait()
            cp_mod(j, 1).wait()

        def cp_wo(j):
            n = H * LANE // NWO
            src = wo_hbm.at[pl.ds(pl.multiple_of(j * n, n), n)]
            dst = wo_s.at[pl.ds(pl.multiple_of(j * (n // 2), n // 2), n // 2)].bitcast(BF16)
            return pltpu.make_async_copy(src, dst, wo_sems.at[j])

        cp_x0 = copy(x_hbm.at[pl.ds(0, P)], x_s.at[pl.ds(PAD, P)])
        late = [copy(w1_hbm, w1_s.bitcast(BF16)),
                copy(x_hbm.at[pl.ds(P, S - P)], x_s.at[pl.ds(PAD + P, S - P)]),
                copy(w2_hbm, w2_s.bitcast(BF16))]
        cp_mlp = [copy(w3_hbm.at[:, pl.ds(j * LANE, LANE)], w3_s.at[j].bitcast(BF16)) for j in range(2 * NT)]
        cp_mlp += [copy(w4_hbm.at[:, pl.ds(j * LANE, LANE)], w4_s.at[j].bitcast(BF16)) for j in range(2 * NH)]

        cp_x0.start()
        cp_w(0).start()
        start_mod(0)

        cv = jnp.broadcast_to(c_ref[...].astype(F32), (8, D))
        silu_c = cv * jax.nn.sigmoid(cv)

        def mod(i):
            if i < 2:
                return jnp.concatenate([mod_s[j, pl.ds(0, 1), pl.ds(i * DK, DK)] for j in range(NKB)], axis=1)
            n = D // MP
            return jnp.concatenate([mod_s[i * n + j, pl.ds(0, 1), :] for j in range(n)], axis=1)

        def after(v, dep):
            dep = pltpu.bitcast(dep[:, -LANE:], U32)
            z = dep[:8]
            for r in range(8, dep.shape[0], 8):
                z = z | dep[r:r + 8]
            z = jnp.tile(z & z_s[...], (v.shape[0] // 8, v.shape[1] // LANE))
            return pltpu.bitcast(pltpu.bitcast(v, U32) | z, v.dtype)

        x_s[pl.ds(0, PAD), :] = jnp.zeros((PAD, D), BF16)
        h_s[pl.ds(0, PAD), :] = jnp.zeros((PAD, D), BF16)
        a_s[...] = jnp.zeros(a_s.shape, F32)
        z_s[...] = jnp.zeros(z_s.shape, U32)
        g_s[pl.ds(G0 + S, 8), :] = jnp.zeros((8, D), F32)

        def zero_g(i):
            g_s[pl.ds(pl.multiple_of(i * SEG, SEG), SEG), :] = jnp.zeros((SEG, D), F32)
        _loop((G0 + S) // SEG, zero_g)

        def relayout(pc, u, tie=None):
            d0, hg = (u // 2) * 16, u % 2
            v = stage_s[pc % NST, pl.ds(d0, 16), pl.ds(hg * 8, 8), :]
            if tie is not None:
                v = v | tie[None]
            v = v.reshape(8, 2, 8, LANE)
            a, b = v[:, 0], v[:, 1]
            lo = (a & 0xFFFF) | (b << 16)
            hi = (a >> 16) | (b & np.uint32(0xFFFF0000))
            t0 = (u % 4) * 144
            for q in range(8):
                t_s[pl.ds(t0 + q * 9, 8), :] = lo[q]
                t_s[pl.ds(t0 + 72 + q * 9, 8), :] = hi[q]
            rows = pl.ds(pl.multiple_of((pc % NKB) * (DK // 2) + d0 // 2, 8), 8)
            head = (pc // NKB) * H + hg * 16
            for j in range(8):
                wqkv_s[head + 2 * j, rows, :] = t_s[pl.ds(t0 + j, 8, stride=9), :]
                wqkv_s[head + 2 * j + 1, rows, :] = t_s[pl.ds(t0 + 72 + j, 8, stride=9), :]

        def mod_cols(j, b):
            cols = pl.ds(b * LANE, LANE)
            mod_s[j, :, cols] = _dot(silu_c, _bf(wmod_s[j, :, cols]))

        def modulate(j):
            wait_mod(j)
            for b in range(MP // LANE):
                mod_cols(j, b)
            m = mod_s[j, pl.ds(0, 1), :]
            for r in range(0, P, 64):
                h0_s[j, pl.ds(r // 2, 32), :] = _pk(n0_s[j, pl.ds(r, 64), :] * (1.0 + m[:, DK:]) + m[:, :DK])

        def norm_ahead(i):
            r = pl.multiple_of(i * LANE, LANE)
            n = _ln(x_s[pl.ds(pl.multiple_of(PAD + r, SEG), LANE), :].astype(F32))
            for j in range(NKB):
                n0_s[j, pl.ds(r, LANE), :] = n[:, j * DK:(j + 1) * DK]

        def ahead(pc):
            @pl.when(pc < 2)
            def _():
                cp_w(pc).wait()
                for u in range(NU):
                    relayout(pc, u)
            pl.when(pc < NKB)(lambda: modulate(pc))
            more = (pc > 0) & (pc + 1 < NPC)
            nxt = jnp.where(more, pc + 1, pc)
            pl.when(more)(lambda: cp_w(nxt).wait())
            pl.when(pc >= NKB)(lambda: wait_mod(pc))
            pl.when(pc == 0)(lambda: cp_w(1).start())
            pl.when(pc + 1 < NPC)(lambda: start_mod(pc + 1))
            start_piece(pc + 2)
            pl.when((pc > 0) & (pc <= NWO))(lambda: cp_wo(pc - 1).start())
            for i, cp in enumerate(late):
                pl.when(pc == NPC - len(late) + i)(cp.start)

            kb = pc % NKB
            rows = pl.ds(pl.multiple_of(kb * (DK // 2), DK // 2), DK // 2)
            for hd in range(H):
                j = (pc // NKB) * H + hd
                for r in range(0, P, LANE):
                    acc = g_s.at[pl.ds(G0 + (hd // NCD) * P + r, LANE), pl.ds((hd % NCD) * LANE, LANE)]
                    y = _dot(_bf(h0_s[kb, pl.ds(r // 2, LANE // 2), :]), _bf(wqkv_s[j, rows, :]))
                    if r == 0:
                        tie = pltpu.bitcast(y[:8], U32) & z_s[...]
                    y = y + jnp.where(kb > 0, acc[...], 0.0)
                    acc[...] = y
                    ring_s[j, pl.ds(OFF + r, LANE), :] = y.astype(BF16)
                relayout(nxt, hd, tie)
                if hd % 8 == 4:
                    mod_cols(pc, hd // 8)

        cp_x0.wait()
        _loop(P // LANE, norm_ahead)
        _loop(NPC, ahead)
        for cp in late + [cp_wo(j) for j in range(NWO)]:
            cp.wait()
        for cp in cp_mlp:
            cp.start()

        def seg_rows(base, j, align=SEG):
            r = base + j * SEG
            return r if isinstance(r, int) else pl.multiple_of(r, align)

        def next_tokens(s):
            r = PAD + P + s * R
            xv = x_s[pl.ds(r if isinstance(r, int) else pl.multiple_of(r, 8), R), :].astype(F32)
            t = _ln(xv) * (1.0 + mod(1)) + mod(0)
            tok_s[...] = t
            return t

        def post_attention(j, r0=0, n=SEG, tie=None):
            r = seg_rows(PAD + r0, j, 16)
            av = a_s[pl.ds(r0, n), :]
            if tie is not None:
                av = after(av, tie)
            x1 = (x_s[pl.ds(r, n), :].astype(F32) + mod(2) * av).astype(BF16)
            x_s[pl.ds(r, n), :] = x1
            h2 = (_ln(x1.astype(F32)) * (1.0 + mod(4)) + mod(3)).astype(BF16)
            h_s[pl.ds(r, n), :] = h2
            n2 = _pk(_ln(h2.astype(F32)))
            n2_s[pl.ds(r0 // 2, n // 2), :] = n2
            return n2

        def w1_stage(n2, j):
            r = seg_rows(G0, j)
            for n in range(NCD):
                g = _gelu(_dot(_bf(n2), _bf(w1_s[:, pl.ds(n * LANE, LANE)])))
                g_s[pl.ds(r, SEG), pl.ds(n * LANE, LANE)] = jnp.where(j >= 0, g, 0.0)

        def shifted(j):
            r = seg_rows(G0, j)
            parts = []
            for gi, sh in enumerate((-1, 1, -2, 2)):
                gv = g_s[pl.ds(r - 8, SEG + 16), pl.ds(gi * (D // 4), D // 4)]
                parts.append(gv[8 + sh:8 + sh + SEG].astype(BF16))
            return jnp.concatenate(parts, axis=1)

        def w2_stage(gs, j):
            rp = seg_rows(PAD, j)
            y = h_s[pl.ds(rp, SEG), :].astype(F32) + _dot(gs, _bf(w2_s[...]))
            g_s[pl.ds(seg_rows(G0 - 2 * SEG, j), SEG), :] = x_s[pl.ds(rp, SEG), :].astype(F32) + mod(5) * y
            n = _ln(y)
            hs, hd = SEG // 2, D // 2
            if isinstance(j, int):
                ro = j * (SEG // 4)
            else:
                ro = pl.multiple_of(jnp.maximum(j, 0) * (SEG // 4), SEG // 4)
            for i, op in enumerate(_strassen_lhs(n[:hs, :hd], n[:hs, hd:], n[hs:, :hd], n[hs:, hd:])):
                wmod_s[i, pl.ds(ro, SEG // 4), :] = _pk(op)
            return n

        row = jax.lax.broadcasted_iota(jnp.int32, (L, L), 0)
        col = jax.lax.broadcasted_iota(jnp.int32, (L, L), 1)

        def step(s):
            mask = (row >= SEG) | (col >= SEG) | (row >= col)
            wpos = pl.multiple_of(jax.lax.rem(s * R, RING), 8)
            rpos = pl.multiple_of(jax.lax.rem(s * SEG + OFF, RING), SEG)
            lhs = jnp.concatenate([tok_s[...], mem_s[...]], axis=0).astype(BF16)

            def proj(j):
                y = _dot(lhs, _bf(wqkv_s[j]))
                ring_s[j, pl.ds(wpos, R), :] = y[:R].astype(BF16)
                return y[R:]

            def full(j, m, dt=F32):
                return jnp.concatenate([ring_s[j, pl.ds(rpos, SEG), :].astype(dt), m.astype(dt)], axis=0)

            qs, ks, vs, ps, side = {}, {}, {}, {}, {}
            for i in range(H + LAG_PV):
                if i < H:
                    qm = proj(i)
                    if i in side:
                        qm = after(qm, side.pop(i))
                    if i == 0:
                        side[i + 6] = post_attention(s - 1, 0, SEG // 2)
                    if i == 7:
                        side[i + 6] = post_attention(s - 1, SEG // 2, SEG // 2, qm)
                    if i == 14:
                        side[i + 6] = next_tokens(jnp.minimum(s + 1, NSEG - 1))
                    if i == 22:
                        gs = shifted(s - LAG_W2)
                        side[i + 2] = pltpu.bitcast(gs, U32)
                if 0 <= i - LAG_QK < H:
                    hq = i - LAG_QK
                    sc = jnp.where(mask, _dot_nt(qs.pop(hq), ks.pop(hq)) * scale, -1e9)
                    e = jnp.exp(sc - jnp.max(sc, axis=-1, keepdims=True))
                    den = jnp.sum(e, axis=-1, keepdims=True)
                    ps[hq] = e * pltpu.reciprocal(den, full_range=False)
                if i < H:
                    km = proj(H + i)
                    qs[i] = full(i, qm)
                    ks[i] = full(H + i, km, BF16)
                if 0 <= i - LAG_V < H:
                    hv = i - LAG_V
                    vs[hv] = full(2 * H + hv, proj(2 * H + hv))
                if i == H + LAG_V:
                    ln_y = w2_stage(gs, s - LAG_W2)
                if 0 <= i - LAG_PV < H:
                    hp = i - LAG_PV
                    o_s[:, pl.ds(hp * LANE, LANE)] = _dot(ps.pop(hp), vs.pop(hp))
            for j in range(NCD):
                ov = o_s[...]
                if j == 2:
                    ov = jnp.concatenate([after(ov[:, :LANE], ln_y), ov[:, LANE:]], axis=1)
                y = _dot(ov, _bf(wo_s[:, pl.ds(j * LANE, LANE)]))
                a_s[:, pl.ds(j * LANE, LANE)] = y[:SEG]
                mem_s[:, pl.ds(j * LANE, LANE)] = y[SEG:]
            w1_stage(n2_s[...], s - 1)

        next_tokens(0)
        mem_s[...] = mem0_ref[...].astype(F32)
        _loop(NSEG, step, unroll=2)
        n2 = post_attention(NSEG - 1)
        w2_stage(shifted(NSEG - 3), NSEG - 3)
        w1_stage(n2, NSEG - 1)
        w2_stage(shifted(NSEG - 2), NSEG - 2)
        w2_stage(shifted(NSEG - 1), NSEG - 1)

        for cp in cp_mlp:
            cp.wait()

        def u_op(i, t):
            return wqkv_s.at[i * 16 + t] if i < 6 else u7_s.at[t]

        def rhs_ops(w, n1, n2, kh):
            b11, b12 = w.at[n1, pl.ds(0, kh)], w.at[n2, pl.ds(0, kh)]
            b21, b22 = w.at[n1, pl.ds(kh, kh)], w.at[n2, pl.ds(kh, kh)]
            for r in range(0, kh, 32):
                rows = pl.ds(r, 32)
                blocks = (_bf(b[rows, :]).astype(F32) for b in (b11, b12, b21, b22))
                for i, v in enumerate(_strassen_rhs_sums(*blocks)):
                    ws_s[i, rows, :] = _pk(v)
            sm = [ws_s.at[i, pl.ds(0, kh)] for i in range(5)]
            return [sm[0], b11, sm[1], sm[2], b22, sm[3], sm[4]]

        def mlp1(t):
            b = rhs_ops(w3_s, t, NT + t, D // 4)
            for r in range(0, S // 2, LANE):
                rows = pl.ds(r // 2, LANE // 2)
                c = _strassen(lambda i: _dot(_bf(wmod_s[i, rows, :]), _bf(b[i][...])))
                for i, op in enumerate(_strassen_lhs(*map(_gelu, c))):
                    u_op(i, t)[rows, :] = _pk(op)

        def cp_out(it, half):
            rows = pl.ds(pl.multiple_of((it // NH) * BM, BM), BM)
            cols = pl.ds(pl.multiple_of((it % NH + half * NH) * LANE, LANE), LANE)
            slot = (it % 2) * 2 + half
            return pltpu.make_async_copy(ob_s.at[slot], out_hbm.at[rows, cols], o_sems.at[slot])

        def mlp2(it):
            @pl.when(it > 1)
            def _():
                cp_out(it - 2, 0).wait()
                cp_out(it - 2, 1).wait()
            blk, n = it // NH, it % NH
            b = rhs_ops(w4_s, n, NH + n, F // 4)
            rows = pl.ds(pl.multiple_of(blk * (BM // 4), BM // 4), BM // 4)

            def prod(i):
                lhs = jnp.concatenate([_bf(u_op(i, t)[rows, :]) for t in range(NT)], axis=1)
                return _dot(lhs, _bf(b[i][...]))
            c11, c12, c21, c22 = _strassen(prod)
            for half, (top, bot) in enumerate(((c11, c21), (c12, c22))):
                cols = pl.ds(pl.multiple_of((n + half * NH) * LANE, LANE), LANE)
                hs = SEG // 2
                y = jnp.concatenate([v[q:q + hs] for q in range(0, BM // 2, hs) for v in (top, bot)], axis=0)
                base = g_s[pl.ds(pl.multiple_of(G0 - 2 * SEG + blk * BM, SEG), BM), cols]
                ob_s[(it % 2) * 2 + half] = (base + gb_s[n + half * NH, pl.ds(0, 1), :] * y).astype(BF16)
            cp_out(it, 0).start()
            cp_out(it, 1).start()

        _loop(NT, mlp1, unroll=2)
        for n in range(NCD):
            gb_s[n] = jnp.broadcast_to(mod(5)[:, n * LANE:(n + 1) * LANE], (8, LANE))
        n_it = (S // BM) * NH
        _loop(n_it, mlp2)
        for it in (n_it - 2, n_it - 1):
            cp_out(it, 0).wait()
            cp_out(it, 1).wait()

    scratch = [
        pltpu.VMEM((PAD + S, D), BF16),
        pltpu.VMEM((PAD + S, D), BF16),
        pltpu.VMEM((NKB, P // 2, DK), U32),
        pltpu.VMEM((3 * H, D // 2, LANE), U32),
        pltpu.VMEM((H * LANE // 2, D), U32),
        pltpu.VMEM((D // 2, D), U32),
        pltpu.VMEM((D // 2, D), U32),
        pltpu.VMEM((2 * NT, D // 2, LANE), U32),
        pltpu.VMEM((2 * NH, F // 2, LANE), U32),
        pltpu.VMEM((NPC, D // 2, MP), U32),
        pltpu.VMEM((NST, DK, H // 2, LANE), U32),
        pltpu.VMEM((3 * H, RING, LANE), BF16),
        pltpu.VMEM((NPC, 8, MP), F32),
        pltpu.VMEM((R, D), F32),
        pltpu.VMEM((M, D), F32),
        pltpu.VMEM((L, H * LANE), F32),
        pltpu.VMEM((SEG, D), F32),
        pltpu.VMEM((SEG // 2, D), U32),
        pltpu.VMEM((G0 + S + 8, D), F32),
        pltpu.VMEM((NKB, P, DK), F32),
        pltpu.VMEM((5, F // 4, LANE), U32),
        pltpu.VMEM((NT, S // 4, LANE), U32),
        pltpu.VMEM((NCD, 8, LANE), F32),
        pltpu.VMEM((4, BM, LANE), BF16),
        pltpu.VMEM((8, LANE), U32),
        pltpu.VMEM((4 * 144 + 16, LANE), U32),
        pltpu.SemaphoreType.DMA((4 + 2 * NT + 2 * NH,)),
        pltpu.SemaphoreType.DMA((NST,)),
        pltpu.SemaphoreType.DMA((2 * NPC,)),
        pltpu.SemaphoreType.DMA((NWO,)),
        pltpu.SemaphoreType.DMA((4,)),
    ]
    return kernel, scratch


@functools.partial(jax.jit, static_argnames=("A_seg_len",))
def pallas_adaLN_cond__memory_aug_recurrent_mem_tr__mixer_s_mlp__prompt_kernel(
    A_x: jax.Array,
    A_mem0: jax.Array,
    A_Wq: jax.Array,
    A_Wk: jax.Array,
    A_Wv: jax.Array,
    A_Wo: jax.Array,
    A_seg_len: int,
    B_x: jax.Array,
    B_w1: jax.Array,
    B_w2: jax.Array,
    B_w3: jax.Array,
    B_w4: jax.Array,
    c: jax.Array,
    w_mod: jax.Array,
):
    del B_x
    B, S, D = A_x.shape
    _, H, Dh = A_Wq.shape
    M = A_mem0.shape[1]
    F = B_w3.shape[1]
    assert (B, S, D, H, Dh, M, int(A_seg_len), F) == (1, 2048, 1024, 32, LANE, 8, 32, 3584)
    kernel, scratch = _make_kernel(S, D, H, M, int(A_seg_len), F)
    hbm = pl.BlockSpec(memory_space=pl.ANY)
    vmem = pl.BlockSpec(memory_space=pltpu.VMEM)
    out = pl.pallas_call(
        kernel,
        in_specs=[hbm, vmem, hbm, hbm, hbm, hbm, hbm, hbm, hbm, hbm, vmem, hbm],
        out_specs=hbm,
        out_shape=jax.ShapeDtypeStruct((S, D), A_x.dtype),
        scratch_shapes=scratch,
        compiler_params=pltpu.CompilerParams(
            vmem_limit_bytes=127 * 1024 * 1024,
            flags={"XLA_TPU_EVENLY_DISTRIBUTE_CRITICAL_NODES": True},
        ),
    )(A_x.reshape(S, D), A_mem0.reshape(M, D), A_Wq, A_Wk, A_Wv, A_Wo.reshape(H * Dh, D),
      B_w1, B_w2, B_w3, B_w4, c, w_mod)
    return out.reshape(B, S, D)
```
